```python
import jax
import jax.numpy as jnp

def _softmax(x, axis=-1):
    return jax.nn.softmax(x, axis=axis)
def _gelu(x):
    return jax.nn.gelu(x, approximate=True)
def _silu(x):
    return jax.nn.silu(x)
def _sigmoid(x):
    return jax.nn.sigmoid(x)
def _layernorm(x, axis=-1, eps=1e-5):
    m = jnp.mean(x, axis=axis, keepdims=True)
    v = jnp.var(x, axis=axis, keepdims=True)
    return (x - m) / jnp.sqrt(v + eps)
def _scatter_add(tgt, idx, src, axis=0):
    return tgt.at[idx].add(src)
def _segment_sum(src, seg, n):
    return jax.ops.segment_sum(src, seg, n)
class _Rng:
    def __init__(self, key):
        self._k = key
    def _next(self):
        self._k, sub = jax.random.split(self._k)
        return sub
    def normal(self, shape):
        return jax.random.normal(self._next(), shape, dtype=jnp.bfloat16)
    def randint(self, lo, hi, shape):
        return jax.random.randint(self._next(), shape, lo, hi, dtype=jnp.int32)
    def uniform(self, shape, lo=0.0, hi=1.0):
        return jax.random.uniform(self._next(), shape, jnp.bfloat16, lo, hi)
    def permutation(self, n):
        return jax.random.permutation(self._next(), n)


kernel_name = 'concat_heads__ssm_conv_h3__softmax_full_mha__prompt'

def _fwd_setup_inputs():
    _rng = _Rng(jax.random.key(int.from_bytes(__import__("os").urandom(4), "little")))
    _w = (lambda a: (lambda t: t.astype(jnp.bfloat16) if jnp.issubdtype(t.dtype, jnp.floating) else t)(jnp.asarray(a)))
    def _A_setup():
        B, S, D = 1, 2048, 640
        ks = 4
        return {
            "q": _w((lambda *s: _rng.normal(s) * 0.05)(B, S, D)),
            "k": _w((lambda *s: _rng.normal(s) * 0.05)(B, S, D)),
            "v": _w((lambda *s: _rng.normal(s) * 0.05)(B, S, D)),
            "shift_k": _w((lambda *s: _rng.normal(s) * 0.05)(D, ks) * 0.5),
            "ssm_k": _w((lambda *s: _rng.normal(s) * 0.05)(D, S) * (1.0 / S ** 0.5)),
            "ssm_D": _w((lambda *s: _rng.normal(s) * 0.05)(D)),
        }
    _A_in = _A_setup()

    def _B_setup():
        B, S, D = 1, 2048, 640
        return {
            "x": _w((lambda *s: _rng.normal(s) * 0.05)(B, S, D)),
            "wqkv": _w((lambda *s: _rng.normal(s) * 0.05)(D, 3 * D)),
            "wo": _w((lambda *s: _rng.normal(s) * 0.05)(D, D)),
        }
    _B_in = _B_setup()

    return {
        "A_q": _A_in["q"],
        "A_k": _A_in["k"],
        "A_v": _A_in["v"],
        "A_shift_k": _A_in["shift_k"],
        "A_ssm_k": _A_in["ssm_k"],
        "A_ssm_D": _A_in["ssm_D"],
        "B_x": _B_in["x"],
        "B_wqkv": _B_in["wqkv"],
        "B_wo": _B_in["wo"],
    }

def _fwd_reference(A_q, A_k, A_v, A_shift_k, A_ssm_k, A_ssm_D, B_x, B_wqkv, B_wo):
    def _A_ref(q, k, v, shift_k, ssm_k, ssm_D):
        B, S, D = q.shape
        ks = shift_k.shape[-1]
        k_pad = jnp.pad(k, ((0, 0), (ks - 1, 0), (0, 0)))
        k_shift = jnp.zeros_like(k)
        for t in range(ks):
            k_shift = k_shift + k_pad[:, t:t + S, :] * shift_k[:, ks - 1 - t][None, None, :]
        kv = k_shift * v
        L = 2 * S
        kv_pad = jnp.pad(kv, ((0, 0), (0, S), (0, 0)))
        kf_pad = jnp.pad(ssm_k, ((0, 0), (0, S)))
        kv_f = (lambda x, axes=(-2,-1): jnp.fft.rfft2(x.astype(jnp.float32), axes=axes))(kv_pad[:, None, :, :], axes=(1, 2))
        kf_f = (lambda x, axes=(-2,-1): jnp.fft.rfft2(x.astype(jnp.float32), axes=axes))(kf_pad[:, None, :], axes=(1, 2))
        kf_f = (lambda x, *d: x.transpose(*d))(kf_f, 1, 2, 0)
        y_f = kv_f * kf_f[None, :, :, :]
        y = (lambda x, s, axes=(-2,-1): jnp.fft.irfft2(x, s=s, axes=axes).astype(jnp.bfloat16))(y_f, (1, L), axes=(1, 2))[:, 0, :S, :]
        y = y + kv * ssm_D[None, None, :]
        return q * y

    def _B_ref(x, wqkv, wo):
        B, S, D = x.shape
        H = 32; Dh = D // H
        qkv = (lambda x, *d: x.transpose(*d))((x @ wqkv).reshape(B, S, 3, H, Dh), 2, 0, 3, 1, 4)
        q, k, v = qkv[0], qkv[1], qkv[2]
        scale = Dh ** -0.5
        scores = jnp.einsum("bhqd,bhkd->bhqk", q, k) * scale
        p = _softmax(scores, axis=-1)
        o = jnp.einsum("bhqk,bhkd->bhqd", p, v)
        return (lambda x, *d: x.transpose(*d))(o, 0, 2, 1, 3).reshape(B, S, D) @ wo

    a = _A_ref(A_q, A_k, A_v, A_shift_k, A_ssm_k, A_ssm_D)
    b = _B_ref(B_x, B_wqkv, B_wo)
    return jnp.concatenate([a, b], axis=-1)


def setup_inputs():
    _inp = _fwd_setup_inputs()
    _gk = jax.random.fold_in(jax.random.key(int.from_bytes(__import__("os").urandom(4), "little")), 2**31 - 1)
    _shapes = [[1, 2048, 1280]]
    _dtypes = ['bfloat16']
    _gks = jax.random.split(_gk, len(_shapes))
    _gs = [jax.random.normal(k, s, dtype=jnp.dtype(d)) * 0.05 for k, s, d in zip(_gks, _shapes, _dtypes)]
    _inp["grad_out"] = _gs[0]
    return _inp

def reference(A_q, A_k, A_v, A_shift_k, A_ssm_k, A_ssm_D, B_x, B_wqkv, B_wo, grad_out):
    _const = dict()
    def _f(*_d):
        return _fwd_reference(**{'A_q': _d[0], 'A_k': _d[1], 'A_v': _d[2], 'A_shift_k': _d[3], 'A_ssm_k': _d[4], 'A_ssm_D': _d[5], 'B_x': _d[6], 'B_wqkv': _d[7], 'B_wo': _d[8], **_const})
    _out, _vjp = jax.vjp(_f, A_q, A_k, A_v, A_shift_k, A_ssm_k, A_ssm_D, B_x, B_wqkv, B_wo)
    _grads = _vjp(grad_out)
    _out0 = jnp.asarray(_out)
    return (_out0, *[jnp.asarray(_g) for _g in _grads])
```

```python
import math

import numpy as np
import jax
import jax.numpy as jnp
from jax import lax
import jax.experimental.pallas as pl
import jax.experimental.pallas.tpu as pltpu

f32 = jnp.float32
bf16 = jnp.bfloat16

S = 2048
D = 640
H = 32
DH = 20
KS = 4
C = 128
NB = S // C
TQ = 512
NQ = S // TQ
CK = 128
NC = S // CK
WIN = 24
NP = H // 2
SCALE = DH ** -0.5
LOG2E = math.log2(math.e)
LN2 = math.log(2.0)
SAFE_BOUND = 40.0

NN = (((1,), (0,)), ((), ()))
NT = (((1,), (1,)), ((), ()))


def _dot(a, b, dims=NN):
    return lax.dot_general(a, b, dims, preferred_element_type=f32)


def _dft_mats():
    f = np.arange(C, dtype=np.float64)[:, None]
    u = np.arange(C, dtype=np.float64)[None, :]
    ang = np.pi * (2.0 * f + 1.0) * u / (2.0 * C)
    fwd = np.concatenate([np.cos(ang), -np.sin(ang)], axis=0)
    inv = fwd.T / C
    return fwd.astype(np.float32), inv.astype(np.float32)


def _split3(x):
    hi = x.astype(bf16).astype(f32)
    r = x - hi
    mid = r.astype(bf16).astype(f32)
    lo = (r - mid).astype(bf16).astype(f32)
    return hi, mid, lo


def _kernel(aq_hbm, ak_hbm, av_hbm, shift_ref, ssmk_hbm, ssmd_ref, x_hbm, wqkv_hbm, wo_hbm, g_hbm,
            f_ref, finv_ref,
            out_hbm, gq_hbm, gk_hbm, gv_hbm, gshift_ref, gssmk_hbm, gssmd_ref, gx_hbm, gwqkv_hbm, gwo_hbm,
            x_v, wqkv_v, wo_v, gb_v, ga_v, aq_v, ak_v, av_v, ssmk_v,
            xt_s, dq_s, dk_s, dv_s, ot_s, ysp_s, dxsp_s, dhsp_s, acc_s,
            sem_in, sem_out):

    def cp(src, dst, sem):
        return pltpu.make_async_copy(src, dst, sem)

    c_wqkv = cp(wqkv_hbm, wqkv_v, sem_in.at[0])
    c_x = cp(x_hbm.at[0], x_v, sem_in.at[1])
    c_wo = cp(wo_hbm, wo_v, sem_in.at[2])
    c_gb = cp(g_hbm.at[0, :, D:2 * D], gb_v, sem_in.at[3])
    c_ak = cp(ak_hbm.at[0], ak_v.at[16:16 + S, :], sem_in.at[4])
    c_av = cp(av_hbm.at[0], av_v, sem_in.at[5])
    c_aq = cp(aq_hbm.at[0], aq_v, sem_in.at[6])
    c_ga = cp(g_hbm.at[0, :, 0:D], ga_v, sem_in.at[7])
    c_sk = cp(ssmk_hbm, ssmk_v, sem_in.at[8])

    c_wqkv.start()
    c_x.start()
    ks_s = x_v

    eye = (lax.broadcasted_iota(jnp.int32, (8, KS), 0) == lax.broadcasted_iota(jnp.int32, (8, KS), 1))
    shift_t = _dot(eye.astype(bf16), shift_ref[...], NT)
    ssm_d = ssmd_ref[...].astype(f32)

    def main_scope(wt_s, qt_s, kt_s, vt_s, dot_s, kvg_s, p_s, m_s, wdo_s, dos_s, xsp_s, hsp_s, gsp_s):
        c_wqkv.wait()
        c_wo.start()
        c_gb.start()
        wt_s[...] = wqkv_v[...].T
        c_x.wait()
        c_ak.start()
        c_av.start()
        c_aq.start()
        c_ga.start()
        c_sk.start()
        c_wo.wait()
        c_gb.wait()

        TN = 512

        def proj_body(n, carry):
            qmax, kmax = carry
            c0 = pl.multiple_of(n * TN, TN)
            xc = x_v[pl.ds(c0, TN), :]
            kt = _dot(wt_s[D:2 * D, :], xc, NT).astype(bf16).astype(f32)
            kt_s[:, pl.ds(c0, TN)] = kt
            vt = _dot(wt_s[2 * D:3 * D, :], xc, NT).astype(bf16).astype(f32)
            vt_s[:, pl.ds(c0, TN)] = vt
            ones = jnp.ones((8, TN), f32)
            zeros = jnp.zeros((40, TN), f32)
            for p in range(NP):
                blk = jnp.concatenate(
                    [kt[40 * p:40 * p + 40], ones, vt[40 * p:40 * p + 40], zeros], axis=0).astype(bf16)
                kvg_s[p, pl.ds(c0, TN), :] = blk.T
            qt = (_dot(wt_s[0:D, :], xc, NT) * (SCALE * LOG2E)).astype(bf16).astype(f32)
            qt_s[:, pl.ds(c0, TN)] = qt
            dot_s[:, pl.ds(c0, TN)] = _dot(wo_v[...], gb_v[pl.ds(c0, TN), :], NT)
            xt_s[:, pl.ds(c0, TN)] = xc.T
            z = jnp.zeros((D, TN), f32)
            dq_s[:, pl.ds(c0, TN)] = z
            dk_s[:, pl.ds(c0, TN)] = z
            dv_s[:, pl.ds(c0, TN)] = z
            ot_s[:, pl.ds(c0, TN)] = z
            qa = jnp.max(jnp.abs(qt).reshape(D // 8, 8, TN), axis=0)
            ka = jnp.max(jnp.abs(kt).reshape(D // 8, 8, TN), axis=0)
            return jnp.maximum(qmax, qa), jnp.maximum(kmax, ka)

        qmax, kmax = lax.fori_loop(0, S // TN, proj_body,
                                   (jnp.zeros((8, TN), f32), jnp.zeros((8, TN), f32)))
        bound = jnp.max(qmax) * jnp.max(kmax) * float(DH)

        c_ak.wait()
        c_av.wait()
        c_aq.wait()
        c_ga.wait()
        c_sk.wait()
        ak_v[0:16, :] = jnp.zeros((16, D), bf16)
        fmat = f_ref[...]

        def pre_body(b, dacc):
            r0 = pl.multiple_of(b * C, C)
            kw = ak_v[pl.ds(r0, C + 16), :].astype(f32)
            ksh = kw[16:16 + C] * shift_t[0:1]
            for j in range(1, KS):
                ksh = ksh + kw[16 - j:16 - j + C] * shift_t[j:j + 1]
            ksh_b = ksh.astype(bf16)
            ks_s[pl.ds(r0, C), :] = ksh_b
            kv = (ksh_b.astype(f32) * av_v[pl.ds(r0, C), :].astype(f32)).astype(bf16)
            dy = (ga_v[pl.ds(r0, C), :].astype(f32) * aq_v[pl.ds(r0, C), :].astype(f32)).astype(bf16)
            xsp_s[b] = _dot(fmat, kv)
            gsp_s[b] = _dot(fmat, dy)
            hsp_s[b] = _dot(fmat, ssmk_v[:, pl.ds(r0, C)], NT)
            prod = kv.astype(f32) * dy.astype(f32)
            return dacc + jnp.sum(prod.reshape(C // 8, 8, D), axis=0)

        dacc = lax.fori_loop(0, NB, pre_body, jnp.zeros((8, D), f32))
        gssmd_ref[...] = jnp.sum(dacc, axis=0, keepdims=True).astype(bf16)

        sgn = jnp.where(lax.broadcasted_iota(jnp.int32, (8, 128), 0) % 2 == 0, 1.0, -1.0).astype(f32)

        def conv_unit(u):
            fb = u // 5
            dt = u % 5
            rr = pl.ds(pl.multiple_of(fb * 8, 8), 8)
            ri = pl.ds(pl.multiple_of(C + fb * 8, 8), 8)
            ll = pl.ds(pl.multiple_of(dt * 128, 128), 128)
            xr = [xsp_s[b, rr, ll] for b in range(NB)]
            xi = [xsp_s[b, ri, ll] for b in range(NB)]
            dr = [gsp_s[b, rr, ll] for b in range(NB)]
            di = [gsp_s[b, ri, ll] for b in range(NB)]
            hr = [hsp_s[b, rr, ll] for b in range(NB)]
            hi = [hsp_s[b, ri, ll] for b in range(NB)]
            gr = [hr[0]] + [hr[b] - sgn * hi[b - 1] for b in range(1, NB)]
            gi = [hi[0]] + [hi[b] + sgn * hr[b - 1] for b in range(1, NB)]
            for b in range(NB):
                ar = ai = None
                for d in range(b + 1):
                    tr = gr[d] * xr[b - d] - gi[d] * xi[b - d]
                    ti = gr[d] * xi[b - d] + gi[d] * xr[b - d]
                    ar = tr if ar is None else ar + tr
                    ai = ti if ai is None else ai + ti
                ysp_s[b, rr, ll] = ar.astype(bf16)
                ysp_s[b, ri, ll] = ai.astype(bf16)
            for b in range(NB):
                ar = ai = None
                for d in range(NB - b):
                    tr = gr[d] * dr[b + d] + gi[d] * di[b + d]
                    ti = gr[d] * di[b + d] - gi[d] * dr[b + d]
                    ar = tr if ar is None else ar + tr
                    ai = ti if ai is None else ai + ti
                dxsp_s[b, rr, ll] = ar.astype(bf16)
                dxsp_s[b, ri, ll] = ai.astype(bf16)
            nr = ni = None
            for d in range(NB - 1, -1, -1):
                ar = ai = None
                for b in range(d, NB):
                    tr = xr[b - d] * dr[b] + xi[b - d] * di[b]
                    ti = xr[b - d] * di[b] - xi[b - d] * dr[b]
                    ar = tr if ar is None else ar + tr
                    ai = ti if ai is None else ai + ti
                if nr is None:
                    orr, oi = ar, ai
                else:
                    orr, oi = ar + sgn * ni, ai - sgn * nr
                dhsp_s[d, rr, ll] = orr.astype(bf16)
                dhsp_s[d, ri, ll] = oi.astype(bf16)
                nr, ni = ar, ai

        def conv_body(u, c):
            conv_unit(u)
            return c

        lax.fori_loop(0, (C // 8) * 5, conv_body, 0)

        row24 = lax.broadcasted_iota(jnp.int32, (WIN, TQ), 0)
        row40 = lax.broadcasted_iota(jnp.int32, (40, TQ), 0)
        row8 = lax.broadcasted_iota(jnp.int32, (8, TQ), 0)
        rowk = lax.broadcasted_iota(jnp.int32, (WIN, CK), 0)

        def head_idx(t):
            h = t // NQ
            par = h % 2
            pair = h // 2
            q0 = pl.multiple_of((t % NQ) * TQ, TQ)
            w0 = pl.multiple_of(pair * 40 + par * 16, 8)
            p0 = pl.multiple_of(pair * 40, 8)
            return h, par, pair, q0, w0, p0

        def aug_rows(v):
            hi, mid, lo = _split3(v)
            return jnp.where(row8 == 0, -hi, jnp.where(row8 == 1, -mid, jnp.where(row8 == 2, -lo, 0.0)))

        def make_wq(t, with_max):
            h, par, pair, q0, w0, p0 = head_idx(t)
            qp = qt_s[pl.ds(p0, 40), pl.ds(q0, TQ)]
            msk = (row40 >= par * DH) & (row40 < par * DH + DH)
            qp = jnp.where(msk, qp, 0.0)
            if with_max:
                mrows = aug_rows(m_s[pl.ds(h, 1), pl.ds(q0, TQ)])
            else:
                mrows = jnp.zeros((8, TQ), f32)
            top = jnp.concatenate([qp, mrows], axis=0).astype(bf16)
            return jnp.concatenate([top, jnp.zeros((80, TQ), bf16)], axis=0)

        m_s[...] = jnp.zeros((H, S), f32)

        @pl.when(jnp.logical_not(bound <= SAFE_BOUND))
        def _():
            def max_body(t, c):
                h, par, pair, q0, w0, p0 = head_idx(t)
                wq = make_wq(t, False)

                def inner(ci, m):
                    k0 = pl.multiple_of(ci * 256, 256)
                    s = _dot(kvg_s[pair, pl.ds(k0, 256), :], wq)
                    return jnp.maximum(m, jnp.max(s.reshape(32, 8, TQ), axis=0))

                m = lax.fori_loop(0, S // 256, inner, jnp.full((8, TQ), -jnp.inf, f32))
                m_s[pl.ds(h, 1), pl.ds(q0, TQ)] = jnp.max(m, axis=0, keepdims=True)
                return c

            lax.fori_loop(0, H * NQ, max_body, 0)

        wdo_s[...] = jnp.zeros((48, TQ), bf16)
        dos_s[...] = jnp.zeros((WIN, TQ), f32)
        p_s[...] = jnp.zeros((S, TQ), bf16)

        LAG = 1

        def att_body(it, carry):
            t1 = jnp.minimum(it, H * NQ - 1)
            t2 = jnp.maximum(it - 1, 0)
            h1, par1, pair1, q1, w1, p1 = head_idx(t1)
            h2, par2, pair2, q2, w2, p2 = head_idx(t2)
            wq = make_wq(t1, True)
            wdo = jnp.concatenate([jnp.zeros((32, TQ), bf16), jnp.zeros((8, TQ), bf16), wdo_s[...],
                                   jnp.zeros((40, TQ), bf16)], axis=0)
            dos = dos_s[...]
            msk2 = (row24 >= par2 * 4) & (row24 < par2 * 4 + DH)
            qw = jnp.where(msk2, qt_s[pl.ds(w2, WIN), pl.ds(q2, TQ)], 0.0)
            lrow = (1 - par1) * DH
            onek = rowk == lrow
            st = dict(o=None, dq=None)
            pn = {}
            dsn = {}

            def s_job(c):
                s = _dot(kvg_s[pair1, c * CK:(c + 1) * CK, :], wq)
                p = jnp.exp2(s).astype(bf16)
                p_s[c * CK:(c + 1) * CK, :] = p
                pn[c] = p

            def d_job(c):
                dp = _dot(kvg_s[pair2, c * CK:(c + 1) * CK, :], wdo)
                p = p_s[c * CK:(c + 1) * CK, :]
                dsn[c] = (p.astype(f32) * dp).astype(bf16)

            def o_job(c):
                vw = jnp.where(onek, 1.0, vt_s[pl.ds(w1, WIN), c * CK:(c + 1) * CK])
                r = _dot(vw, pn[c])
                st['o'] = r if st['o'] is None else st['o'] + r

            def q_job(c):
                r = _dot(kt_s[pl.ds(w2, WIN), c * CK:(c + 1) * CK], dsn[c])
                st['dq'] = r if st['dq'] is None else st['dq'] + r

            def v_job(c):
                p = p_s[c * CK:(c + 1) * CK, :]
                dv_s[pl.ds(w2, WIN), c * CK:(c + 1) * CK] += _dot(dos, p, NT)

            def k_job(c):
                dk_s[pl.ds(w2, WIN), c * CK:(c + 1) * CK] += _dot(qw, dsn[c], NT)

            jobs = dict(S=s_job, D=d_job, O=o_job, Q=q_job, V=v_job, K=k_job)
            for c in range(NC + LAG):
                for o in 'DVKSOQ':
                    cc = c if o in 'SDV' else c - LAG
                    if 0 <= cc < NC:
                        jobs[o](cc)

            dq_s[pl.ds(w2, WIN), pl.ds(q2, TQ)] += jnp.where(msk2, st['dq'], 0.0)

            oacc = st['o']
            msk1 = (row24 >= par1 * 4) & (row24 < par1 * 4 + DH)
            l = jnp.sum(jnp.where(row24 == lrow, oacc, 0.0), axis=0, keepdims=True)
            rl = 1.0 / l
            o = jnp.where(msk1, oacc * rl, 0.0)
            ot_s[pl.ds(w1, WIN), pl.ds(q1, TQ)] = jnp.where(msk1, o, ot_s[pl.ds(w1, WIN), pl.ds(q1, TQ)])
            dosn = jnp.where(msk1, dot_s[pl.ds(w1, WIN), pl.ds(q1, TQ)] * rl, 0.0).astype(bf16).astype(f32)
            delta = jnp.sum(dosn * o, axis=0, keepdims=True)
            m40 = (row40 >= par1 * DH) & (row40 < par1 * DH + DH)
            dop = jnp.where(m40, dot_s[pl.ds(p1, 40), pl.ds(q1, TQ)] * rl, 0.0)
            wdo_s[...] = jnp.concatenate([aug_rows(delta), dop], axis=0).astype(bf16)
            dos_s[...] = dosn
            return carry

        lax.fori_loop(0, H * NQ + 1, att_body, 0)

    pl.run_scoped(
        main_scope,
        pltpu.VMEM((3 * D, D), bf16),
        pltpu.VMEM((D, S), f32),
        pltpu.VMEM((D, S), f32),
        pltpu.VMEM((D, S), f32),
        pltpu.VMEM((D, S), f32),
        pltpu.VMEM((NP, S, 128), bf16),
        pltpu.VMEM((S, TQ), bf16),
        pltpu.VMEM((H, S), f32),
        pltpu.VMEM((48, TQ), bf16),
        pltpu.VMEM((WIN, TQ), f32),
        pltpu.VMEM((NB, 2 * C, D), f32),
        pltpu.VMEM((NB, 2 * C, D), f32),
        pltpu.VMEM((NB, 2 * C, D), f32),
    )

    def tail_scope(oa_v, gq_v, gk_v, gv_v, gsk_v, ob_v, gx_v, gw_v, gwo_v, dqkv_s, o_s):
        finv = finv_ref[...]
        acc_s[...] = jnp.zeros((KS, 8, D), f32)

        def post_body(i, nxt):
            b = NB - 1 - i
            r0 = pl.multiple_of(b * C, C)
            rows = pl.ds(r0, C)
            ksh = ks_s[rows, :].astype(f32)
            vv = av_v[rows, :].astype(f32)
            qq = aq_v[rows, :].astype(f32)
            gg = ga_v[rows, :].astype(f32)
            y = _dot(finv, ysp_s[b]) + (ksh * vv) * ssm_d
            oa_v[rows, :] = (qq * y).astype(bf16)
            gq_v[rows, :] = (gg * y).astype(bf16)
            dkv = _dot(finv, dxsp_s[b]) + (gg * qq) * ssm_d
            gv_v[rows, :] = (dkv * ksh).astype(bf16)
            dks = dkv * vv
            ext = jnp.concatenate([dks, nxt], axis=0)
            kk = ak_v[pl.ds(pl.multiple_of(r0 + 16, 16), C), :].astype(f32)
            gk = None
            for j in range(KS):
                sh = ext[j:j + C]
                t = sh * shift_t[j:j + 1]
                gk = t if gk is None else gk + t
                acc_s[j] += jnp.sum((sh * kk).reshape(C // 8, 8, D), axis=0)
            gk_v[rows, :] = gk.astype(bf16)
            gsk_v[:, rows] = _dot(finv, dhsp_s[b]).astype(bf16).T
            return dks[0:8]

        lax.fori_loop(0, NB, post_body, jnp.zeros((8, D), f32))
        o_oa = cp(oa_v, out_hbm.at[0, :, 0:D], sem_out.at[0])
        o_gq = cp(gq_v, gq_hbm.at[0], sem_out.at[1])
        o_gk = cp(gk_v, gk_hbm.at[0], sem_out.at[2])
        o_gv = cp(gv_v, gv_hbm.at[0], sem_out.at[3])
        o_gs = cp(gsk_v, gssmk_hbm, sem_out.at[4])
        o_oa.start()
        o_gq.start()
        o_gk.start()
        o_gv.start()
        o_gs.start()
        r8 = lax.broadcasted_iota(jnp.int32, (8, D), 0)
        gsh = jnp.zeros((8, D), f32)
        for j in range(KS):
            gsh = jnp.where(r8 == j, jnp.sum(acc_s[j], axis=0, keepdims=True), gsh)
        gsh = jnp.concatenate([gsh, jnp.zeros((120, D), f32)], axis=0)
        gshift_ref[...] = gsh.T[:, 0:KS].astype(bf16)

        TN = 512

        def gx_body(n, c):
            c0 = pl.multiple_of(n * TN, TN)
            cols = pl.ds(c0, TN)
            w = jnp.concatenate([(dq_s[:, cols] * SCALE).astype(bf16),
                                 (dk_s[:, cols] * LN2).astype(bf16),
                                 dv_s[:, cols].astype(bf16)], axis=0)
            dqkv_s[:, cols] = w
            gx_v[cols, :] = _dot(wqkv_v[...], w).astype(bf16).T
            ob = ot_s[:, cols].astype(bf16)
            o_s[:, cols] = ob
            ob_v[cols, :] = _dot(ob.T, wo_v[...]).astype(bf16)
            return c

        lax.fori_loop(0, S // TN, gx_body, 0)
        o_gx = cp(gx_v, gx_hbm.at[0], sem_out.at[5])
        o_ob = cp(ob_v, out_hbm.at[0, :, D:2 * D], sem_out.at[6])
        o_gx.start()
        o_ob.start()

        TW = 384

        def gw_body(n, c):
            c0 = pl.multiple_of(n * TW, 128)
            gw_v[:, pl.ds(c0, TW)] = _dot(xt_s[...], dqkv_s[pl.ds(c0, TW), :], NT).astype(bf16)
            return c

        lax.fori_loop(0, 3 * D // TW, gw_body, 0)
        o_gw = cp(gw_v, gwqkv_hbm, sem_out.at[7])
        o_gw.start()
        gwo_v[...] = _dot(o_s[...], gb_v[...]).astype(bf16)
        o_gwo = cp(gwo_v, gwo_hbm, sem_out.at[8])
        o_gwo.start()
        for o in (o_oa, o_gq, o_gk, o_gv, o_gs, o_gx, o_ob, o_gw, o_gwo):
            o.wait()

    pl.run_scoped(
        tail_scope,
        pltpu.VMEM((S, D), bf16),
        pltpu.VMEM((S, D), bf16),
        pltpu.VMEM((S, D), bf16),
        pltpu.VMEM((S, D), bf16),
        pltpu.VMEM((D, S), bf16),
        pltpu.VMEM((S, D), bf16),
        pltpu.VMEM((S, D), bf16),
        pltpu.VMEM((D, 3 * D), bf16),
        pltpu.VMEM((D, D), bf16),
        pltpu.VMEM((3 * D, S), bf16),
        pltpu.VMEM((D, S), bf16),
    )


@jax.jit
def pallas_concat_heads__ssm_conv_h3__softmax_full_mha__prompt_kernel(
    A_q: jax.Array,
    A_k: jax.Array,
    A_v: jax.Array,
    A_shift_k: jax.Array,
    A_ssm_k: jax.Array,
    A_ssm_D: jax.Array,
    B_x: jax.Array,
    B_wqkv: jax.Array,
    B_wo: jax.Array,
    grad_out: jax.Array,
):
    fwd_np, inv_np = _dft_mats()
    fmat = jnp.asarray(fwd_np, dtype=bf16)
    finv = jnp.asarray(inv_np, dtype=bf16)

    hbm = pl.BlockSpec(memory_space=pl.ANY)
    vmem = pl.BlockSpec(memory_space=pltpu.VMEM)
    sds = jax.ShapeDtypeStruct
    out_shape = (
        sds((1, S, 2 * D), bf16),
        sds((1, S, D), bf16),
        sds((1, S, D), bf16),
        sds((1, S, D), bf16),
        sds((D, KS), bf16),
        sds((D, S), bf16),
        sds((1, D), bf16),
        sds((1, S, D), bf16),
        sds((D, 3 * D), bf16),
        sds((D, D), bf16),
    )
    scratch = [
        pltpu.VMEM((S, D), bf16),
        pltpu.VMEM((D, 3 * D), bf16),
        pltpu.VMEM((D, D), bf16),
        pltpu.VMEM((S, D), bf16),
        pltpu.VMEM((S, D), bf16),
        pltpu.VMEM((S, D), bf16),
        pltpu.VMEM((S + 16, D), bf16),
        pltpu.VMEM((S, D), bf16),
        pltpu.VMEM((D, S), bf16),
        pltpu.VMEM((D, S), bf16),
        pltpu.VMEM((D, S), f32),
        pltpu.VMEM((D, S), f32),
        pltpu.VMEM((D, S), f32),
        pltpu.VMEM((D, S), f32),
        pltpu.VMEM((NB, 2 * C, D), bf16),
        pltpu.VMEM((NB, 2 * C, D), bf16),
        pltpu.VMEM((NB, 2 * C, D), bf16),
        pltpu.VMEM((KS, 8, D), f32),
        pltpu.SemaphoreType.DMA((9,)),
        pltpu.SemaphoreType.DMA((9,)),
    ]
    outs = pl.pallas_call(
        _kernel,
        out_shape=out_shape,
        in_specs=[hbm, hbm, hbm, vmem, hbm, vmem, hbm, hbm, hbm, hbm, vmem, vmem],
        out_specs=(hbm, hbm, hbm, hbm, vmem, hbm, vmem, hbm, hbm, hbm),
        scratch_shapes=scratch,
        compiler_params=pltpu.CompilerParams(vmem_limit_bytes=127 * 1024 * 1024),
    )(A_q, A_k, A_v, A_shift_k, A_ssm_k, A_ssm_D.reshape(1, D), B_x, B_wqkv, B_wo, grad_out, fmat, finv)
    outs = list(outs)
    outs[6] = outs[6].reshape(D)
    return tuple(outs)
```

```python
import math

import numpy as np
import jax
import jax.numpy as jnp
from jax import lax
import jax.experimental.pallas as pl
import jax.experimental.pallas.tpu as pltpu

f32 = jnp.float32
bf16 = jnp.bfloat16

S = 2048
D = 640
H = 32
DH = 20
KS = 4
C = 128
NB = S // C
ND = D // 128
TQ = 512
NQ = S // TQ
NT_ALL = H * NQ
CK = 128
NC = S // CK
WIN = 24
NP = H // 2
NU = (C // 8) * ND
SPK = 6
TN = 512
SCALE = DH ** -0.5
LOG2E = math.log2(math.e)
LN2 = math.log(2.0)
SAFE_BOUND = 40.0

NN = (((1,), (0,)), ((), ()))
NT = (((1,), (1,)), ((), ()))


def _dot(a, b, dims=NN):
    return lax.dot_general(a, b, dims, preferred_element_type=f32)


def _dft_mats():
    hf = C // 2
    f = np.concatenate([np.arange(hf), C - 1 - np.arange(hf)]).astype(np.float64)[:, None]
    u = np.arange(C, dtype=np.float64)[None, :]
    ang = np.pi * (2.0 * f + 1.0) * u / (2.0 * C)
    fwd = np.concatenate([np.cos(ang), -np.sin(ang)], axis=0)
    half = np.concatenate([np.cos(ang[:hf]), -np.sin(ang[:hf])], axis=0).T / C
    inv = np.concatenate([half[0::2], half[1::2]], axis=0)
    return fwd.astype(np.float32), inv.astype(np.float32)


def _v8(i):
    return slice(8 * i, 8 * i + 8)


def _kernel(aq_hbm, ak_hbm, av_hbm, shift_hbm, ssmk_hbm, ssmd_hbm, x_hbm, wqkv_hbm, wo_hbm, g_hbm,
            f_hbm, finv_hbm,
            out_hbm, gq_hbm, gk_hbm, gv_hbm, gshift_hbm, gssmk_hbm, gssmd_hbm, gx_hbm, gwqkv_hbm, gwo_hbm,
            x_v, wqkv_v, wo_v, gb_v, ga_v, aq_v, ak_v, av_v, ssmk_v, xt_s,
            qt_s, kt_s, vt_s, dot_s, dk_s, dv_s, kvg_s, pa_s, pb_s, pc_s, pd_s,
            ysp_s, dxsp_s, dhsp_s, sp_s, m_s,
            wdo_s, dos_s, acc_s, dsc_s, f_ref, finv_ref, sacc_s, shift_ref, ssmd_ref,
            zero_s, sem_in, sem_out):

    def cp(src, dst, sem):
        return pltpu.make_async_copy(src, dst, sem)

    def c_x(n):
        r = pl.ds(pl.multiple_of(n * TN, TN), TN)
        return cp(x_hbm.at[0, r, :], x_v.at[r, :], sem_in.at[8 + n])

    def c_gb(n):
        r = pl.ds(pl.multiple_of(n * TN, TN), TN)
        return cp(g_hbm.at[0, r, D:2 * D], gb_v.at[r, :], sem_in.at[12 + n])

    def c_w(j):
        cols = pl.ds(pl.multiple_of(j * D, 128), D)
        return cp(wqkv_hbm.at[:, cols], wqkv_v.at[:, cols], sem_in.at[16 + j])

    c_wo = cp(wo_hbm, wo_v, sem_in.at[1])
    c_ak = cp(ak_hbm.at[0], ak_v, sem_in.at[2])
    c_av = cp(av_hbm.at[0], av_v, sem_in.at[3])
    c_aq = cp(aq_hbm.at[0], aq_v, sem_in.at[4])
    c_ga = cp(g_hbm.at[0, :, 0:D], ga_v, sem_in.at[5])
    c_sk = cp(ssmk_hbm, ssmk_v, sem_in.at[6])
    c_small = [cp(shift_hbm, shift_ref, sem_in.at[19]), cp(ssmd_hbm, ssmd_ref, sem_in.at[20]),
               cp(f_hbm, f_ref, sem_in.at[21]), cp(finv_hbm, finv_ref, sem_in.at[22])]

    c_gb(0).start()
    c_wo.start()
    for n in range(3):
        c_gb(n + 1).start()
        c_w(n).start()
    for n in range(S // TN):
        c_x(n).start()
    for cc in c_small + [c_sk, c_ga, c_aq, c_ak, c_av]:
        cc.start()

    wt_s = dxsp_s
    ks_s = x_v
    dq_s = qt_s
    ot_s = dot_s

    def zero_body(n, c):
        cols = pl.ds(pl.multiple_of(n * 128, 128), 128)
        dk_s[:, cols] = jnp.zeros((D, 128), f32)
        dv_s[:, cols] = jnp.zeros((D, 128), f32)
        m_s[:, cols] = jnp.zeros((H * 8, 128), f32)
        return c

    lax.fori_loop(0, S // 128, zero_body, 0)
    dsc_s[...] = jnp.zeros((CK, TQ), bf16)
    acc_s[...] = jnp.zeros((2 * NQ, WIN, TQ), f32)
    sacc_s[...] = jnp.zeros((KS + 1, 8, D), f32)
    zero_s[0] = 0

    def do_chunk(n):
        cols = pl.ds(pl.multiple_of(n * TN, TN), TN)
        dot_s[:, cols] = _dot(wo_v[...], gb_v[cols, :], NT)

    c_wo.wait()
    c_gb(0).wait()
    do_chunk(0)

    def do_body(n, c):
        c_gb(n).wait()
        c_w(n - 1).wait()

        do_chunk(n)
        w0 = pl.multiple_of((n - 1) * D, 128)
        wt_s[pl.ds(w0, D), :] = wqkv_v[:, pl.ds(w0, D)].T
        return c

    lax.fori_loop(1, S // TN, do_body, 0)

    def proj_body(n, carry):
        qmax, kmax = carry
        c_x(n).wait()

        c0 = pl.multiple_of(n * TN, TN)
        xc = x_v[pl.ds(c0, TN), :]
        kt = _dot(wt_s[D:2 * D, :], xc, NT).astype(bf16).astype(f32)
        kt_s[:, pl.ds(c0, TN)] = kt
        vt = _dot(wt_s[2 * D:3 * D, :], xc, NT).astype(bf16).astype(f32)
        vt_s[:, pl.ds(c0, TN)] = vt
        ones = jnp.ones((8, TN), f32)
        zeros = jnp.zeros((40, TN), f32)
        for p in range(NP):
            blk = jnp.concatenate(
                [kt[40 * p:40 * p + 40], ones, vt[40 * p:40 * p + 40], zeros], axis=0).astype(bf16)
            kvg_s[p, pl.ds(c0, TN), :] = blk.T
        qt = (_dot(wt_s[0:D, :], xc, NT) * (SCALE * LOG2E)).astype(bf16).astype(f32)
        qt_s[:, pl.ds(c0, TN)] = qt
        xt_s[:, pl.ds(c0, TN)] = xc.T
        qa = jnp.max(jnp.abs(qt).reshape(D // 8, 8, TN), axis=0)
        ka = jnp.max(jnp.abs(kt).reshape(D // 8, 8, TN), axis=0)
        return jnp.maximum(qmax, qa), jnp.maximum(kmax, ka)

    qmax, kmax = lax.fori_loop(0, S // TN, proj_body,
                               (jnp.zeros((8, TN), f32), jnp.zeros((8, TN), f32)))
    bound = jnp.max(qmax) * jnp.max(kmax) * float(DH)

    c_ak.wait()
    c_av.wait()
    c_aq.wait()
    c_ga.wait()
    c_sk.wait()
    for cc in c_small:
        cc.wait()

    def lanes(dt):
        return slice(dt * 128, (dt + 1) * 128)

    PRU = 8

    def pre_chunk(i, k):
        fmat = f_ref[...]
        taps = shift_ref[...].astype(f32)
        grp = pl.ds(pl.multiple_of(i * PRU * C, PRU * C), PRU * C)
        rows = slice(k * C, (k + 1) * C)
        av, aq, ga, ak, ks = (r.at[grp, :] for r in (av_v, aq_v, ga_v, ak_v, ks_s))
        spv = sp_s.at[:, pl.ds(pl.multiple_of(i * PRU * SPK * 8, PRU * SPK * 8), PRU * SPK * 8), :]

        def put(kk, dt, val):
            for part in range(2):
                spv[dt * 16:(dt + 1) * 16, _v8(SPK * k + 2 * kk + part), :] = (
                    val[part * C:(part + 1) * C, :].reshape(C // 8, 8, 128))

        hs = _dot(fmat, ssmk_v.at[:, grp][:, rows], NT)
        for dt in range(ND):
            put(1, dt, hs[:, lanes(dt)])
        for dt in range(ND):
            ln = lanes(dt)
            dy = (ga[rows, ln].astype(f32) * aq[rows, ln].astype(f32)).astype(bf16)
            put(2, dt, _dot(fmat, dy))
            kf = ak[rows, ln].astype(f32)
            if k == 0:
                h0 = pl.multiple_of(jnp.maximum(i * PRU * C - 16, 0), 16)
                halo = jnp.where(i > 0, ak_v[pl.ds(h0, 16), ln].astype(f32)[8:16], 0.0)
            else:
                halo = ak[k * C - 16:k * C, ln].astype(f32)[8:16]
            ext = jnp.concatenate([halo, kf], axis=0)
            ksh = kf * taps[0:1, ln]
            for j in range(1, KS):
                ksh = ksh + pltpu.roll(ext, j, 0)[8:8 + C] * taps[j:j + 1, ln]
            ks[rows, ln] = ksh.astype(bf16)
            put(0, dt, _dot(fmat, (ksh * av[rows, ln].astype(f32)).astype(bf16)))

    def pre_body(i, c):
        for k in range(PRU):
            pre_chunk(i, k)
        return c

    lax.fori_loop(0, NB // PRU, pre_body, 0)
    ssm_d = ssmd_ref[...].astype(f32).reshape(1, D)
    for dt in range(ND):
        sp_s[dt * 16:(dt + 1) * 16, _v8(2), :] += ssm_d[:, lanes(dt)].reshape(1, 1, 128)

    def conv_ops(k, mirror):
        sgn = jnp.where(lax.broadcasted_iota(jnp.int32, (8, 128), 0) % 2 == mirror, 1.0, -1.0).astype(f32)
        dt = lax.shift_right_logical(k, 3)
        u = dt * 16 + (k & 7) + 8 * mirror
        r0 = pl.multiple_of((k & 7) * 8, 8)
        ll = pl.ds(pl.multiple_of(dt * 128, 128), 128)
        ops = []

        def ld(kb):
            k, b = kb
            return sp_s[u, _v8(SPK * b + 2 * k), :], sp_s[u, _v8(SPK * b + 2 * k + 1), :]

        def cm(a, b, conj):
            if conj:
                return a[0] * b[0] + a[1] * b[1], a[0] * b[1] - a[1] * b[0]
            return a[0] * b[0] - a[1] * b[1], a[0] * b[1] + a[1] * b[0]

        def st(ref, b, vr, vi):
            j = 2 * (ref[1] * NB + b)
            if not mirror:
                sp_s[NU + 1, _v8(j), :] = vr
                sp_s[NU + 1, _v8(j + 1), :] = vi
            else:
                zr, zi = sp_s[NU + 1, _v8(j), :], sp_s[NU + 1, _v8(j + 1), :]
                for q, v in enumerate((zr + vr, zi - vi, zr - vr, zi + vi)):
                    ref[0][pl.ds(pl.multiple_of(r0 + b * 2 * C + q * (C // 2), 8), 8), ll] = v.astype(bf16)

        def add_group(outs, conj):
            accs = [None] * len(outs)
            cache = {}
            nt = max(len(t) for t, _ in outs)

            def mk(i):
                def op():
                    a = None
                    newc = {}
                    for oi, (terms, _) in enumerate(outs):
                        if i >= len(terms):
                            continue
                        ka, kb = terms[i]
                        if a is None:
                            a = ld(ka)
                        b = cache[kb] if kb in cache else ld(kb)
                        newc[kb] = b
                        t = cm(a, b, conj)
                        accs[oi] = t if accs[oi] is None else (accs[oi][0] + t[0], accs[oi][1] + t[1])
                    cache.clear()
                    cache.update(newc)
                    if i == nt - 1:
                        for oi, (_, fin) in enumerate(outs):
                            fin(*accs[oi])
                return op

            for i in range(nt):
                ops.append((sum(1 for t, _ in outs if i < len(t)), mk(i)))

        def fin_next(ref):
            prev = {}

            def mkfin(d):
                def fin(ar, ai):
                    if d > 0:
                        st(ref, d - 1, prev['r'] + sgn * ai, prev['i'] - sgn * ar)
                    if d == NB - 1:
                        st(ref, d, ar, ai)
                    prev['r'], prev['i'] = ar, ai
                return fin
            return mkfin

        def fin_prev(ref):
            prev = {}

            def mkfin(b):
                def fin(ar, ai):
                    if b > 0:
                        st(ref, b, ar - sgn * prev['i'], ai + sgn * prev['r'])
                    else:
                        st(ref, b, ar, ai)
                    prev['r'], prev['i'] = ar, ai
                return fin
            return mkfin

        X, G, Y = 0, 1, 2
        BLK = 2
        fh, fy, fx = fin_next((dhsp_s, 0)), fin_prev((ysp_s, 1)), fin_next((dxsp_s, 2))
        for d0 in range(0, NB, BLK):
            add_group([([((X, j), (Y, j + d)) for j in range(NB - d)], fh(d))
                       for d in range(d0, d0 + BLK)], True)
        for b0 in range(0, NB, BLK):
            add_group([([((G, d), (X, b - d)) for d in range(b + 1)], fy(b))
                       for b in range(b0, b0 + BLK)], False)
        for b0 in range(0, NB, BLK):
            add_group([([((G, d), (Y, b + d)) for d in range(NB - b)], fx(b))
                       for b in range(b0, b0 + BLK)], True)
        return ops

    def make_pacer(extra, npts):
        tot = sum(w for w, _ in extra)
        zero = zero_s[0]
        sink_u = zero + NU
        sink_r = pl.ds(pl.multiple_of(zero, 8), 8)
        pos = dict(i=0, w=0, pt=0)

        def tick(val, r):
            pos['pt'] += 1
            lim = pos['pt'] * tot / npts
            if pos['i'] < len(extra) and pos['w'] < lim:
                sp_s[sink_u, sink_r, :] = val[r:r + 8, 0:128]
            while pos['i'] < len(extra) and pos['w'] < lim:
                w, op = extra[pos['i']]
                op()
                pos['i'] += 1
                pos['w'] += w

        return tick

    def iota(n, m):
        return lax.broadcasted_iota(jnp.int32, (n, m), 0)

    def head_idx(h):
        if isinstance(h, int):
            par, pair = h % 2, h // 2
            return par, pair, pair * 40 + par * 16, pair * 40, h * 8
        par = h & 1
        pair = lax.shift_right_logical(h, 1)
        return (par, pair, pl.multiple_of(pair * 40 + par * 16, 8), pl.multiple_of(pair * 40, 8),
                pl.multiple_of(h * 8, 8))

    def make_wq(h, qcols):
        par, pair, w0, p0, m0 = head_idx(h)
        row40 = iota(40, TQ)
        qp = qt_s[pl.ds(p0, 40), qcols]
        qp = jnp.where((row40 >= par * DH) & (row40 < par * DH + DH), qp, 0.0)
        top = jnp.concatenate([qp, m_s[pl.ds(m0, 8), qcols]], axis=0).astype(bf16)
        return jnp.concatenate([top, jnp.zeros((80, TQ), bf16)], axis=0)

    @pl.when(jnp.logical_not(bound <= SAFE_BOUND))
    def _():
        def max_body(t, c):
            h = lax.shift_right_logical(t, 2)
            par, pair, w0, p0, m0 = head_idx(h)
            qcols = pl.ds(pl.multiple_of((t & 3) * TQ, TQ), TQ)
            wq = make_wq(h, qcols)

            def inner(ci, m):
                k0 = pl.multiple_of(ci * 256, 256)
                s = _dot(kvg_s[pair, pl.ds(k0, 256), :], wq)
                return jnp.maximum(m, jnp.max(s.reshape(32, 8, TQ), axis=0))

            m = lax.fori_loop(0, S // 256, inner, jnp.full((8, TQ), -jnp.inf, f32))
            nm = -jnp.max(m, axis=0, keepdims=True)
            hi = nm.astype(bf16).astype(f32)
            mid = (nm - hi).astype(bf16).astype(f32)
            lo = nm - hi - mid
            row8 = iota(8, TQ)
            m_s[pl.ds(m0, 8), qcols] = jnp.where(
                row8 == 0, hi, jnp.where(row8 == 1, mid, jnp.where(row8 == 2, lo, 0.0)))
            return c

        lax.fori_loop(0, NT_ALL, max_body, 0)

    def rows_of(c):
        return slice(c * CK, (c + 1) * CK)

    P_S = (pa_s, pb_s, pc_s, pd_s)

    def fwd_ctx(h, sid):
        par, pair, w0, p0, m0 = head_idx(h)
        p_s = P_S[sid]
        acc_ref = acc_s.at[sid]
        lz = {}
        onek = iota(WIN, CK) == (1 - par) * DH
        pn = {}

        def s_job(c, hook):
            if 'wq' not in lz:
                lz['wq'] = make_wq(h, slice(sid * TQ, (sid + 1) * TQ))
            s = _dot(kvg_s[pair, rows_of(c), :], lz['wq'])
            hook(s)
            p = jnp.exp2(s).astype(bf16)
            p_s[rows_of(c), :] = p
            pn[c] = p

        def o_job(c):
            vw = jnp.where(onek, 1.0, vt_s[pl.ds(w0, WIN), rows_of(c)])
            r = _dot(vw, pn[c] if c in pn else p_s[rows_of(c), :])
            if c == 0:
                acc_ref[...] = r
            elif c < NC - 1:
                acc_ref[...] += r
            else:
                oacc = acc_ref[...] + r
                for qt in range(TQ // 128):
                    o0 = (sid * 4 + qt) * WIN
                    sp_s[NU + 2, o0:o0 + WIN, :] = oacc[:, lanes(qt)]

        def fin_op(qt):
            def op():
                row24 = iota(WIN, 128)
                row8 = iota(8, 128)
                o0 = (sid * 4 + qt) * WIN
                oacc = sp_s[NU + 2, o0:o0 + WIN, :]
                cs = slice(sid * TQ + qt * 128, sid * TQ + (qt + 1) * 128)
                msk = (row24 >= par * 4) & (row24 < par * 4 + DH)
                l = jnp.where(par == 0, oacc[DH:DH + 1], oacc[0:1])
                rl = 1.0 / l
                o = oacc * rl
                dow = dot_s[pl.ds(w0, WIN), cs]
                dosn = jnp.where(msk, dow * rl, 0.0).astype(bf16).astype(f32)
                nd = -jnp.sum(dosn * o, axis=0, keepdims=True)
                hi = nd.astype(bf16).astype(f32)
                drows = jnp.where(row8 == 0, hi, jnp.where(row8 == 1, nd - hi, 0.0))
                z8 = jnp.zeros((8, 128), f32)
                z16 = jnp.zeros((16, 128), f32)
                dop = jnp.where(par == 0, jnp.concatenate([dosn, z16], axis=0),
                                jnp.concatenate([z16, dosn], axis=0))
                wdo_s[sid, :, lanes(qt)] = jnp.concatenate([z8, drows, dop, z8], axis=0).astype(bf16)
                dos_s[sid, :, lanes(qt)] = dosn
                ot_s[pl.ds(w0, WIN), cs] = jnp.where(msk, o, dow)
            return op

        return dict(S=s_job, O=o_job, fin=[fin_op(qt) for qt in range(TQ // 128)])

    def bwd_ctx(h, sid, valid=None):
        par, pair, w0, p0, m0 = head_idx(h)
        p_s = P_S[sid]
        acc_ref = acc_s.at[NQ + sid]
        qcols = slice(sid * TQ, (sid + 1) * TQ)
        row24 = iota(WIN, TQ)
        msk = (row24 >= par * 4) & (row24 < par * 4 + DH)
        lz = {}
        dsn = {}

        def d_job(c, hook):
            if 'wdo' not in lz:
                z32 = jnp.zeros((32, TQ), bf16)
                lz['wdo'] = jnp.concatenate([z32, wdo_s[sid], z32], axis=0)
            dp = _dot(kvg_s[pair, rows_of(c), :], lz['wdo'])
            hook(dp)
            dsn[c] = (p_s[rows_of(c), :].astype(f32) * dp).astype(bf16)

        def getds(c):
            return dsn[c] if c in dsn else dsc_s[...]

        def q_job(c):
            r = _dot(kt_s[pl.ds(w0, WIN), rows_of(c)], getds(c))
            if c == 0:
                acc_ref[...] = r
            elif c < NC - 1:
                acc_ref[...] += r
            else:
                mk = msk if valid is None else (msk & valid)
                dq_s[pl.ds(w0, WIN), qcols] = jnp.where(mk, acc_ref[...] + r, dq_s[pl.ds(w0, WIN), qcols])

        def v_job(c):
            if 'dos' not in lz:
                lz['dos'] = dos_s[sid]
            dv_s[pl.ds(w0, WIN), rows_of(c)] += _dot(lz['dos'], p_s[rows_of(c), :], NT)

        def k_job(c):
            if 'qw' not in lz:
                lz['qw'] = jnp.where(msk, qt_s[pl.ds(w0, WIN), qcols], 0.0)
            dk_s[pl.ds(w0, WIN), rows_of(c)] += _dot(lz['qw'], getds(c), NT)

        def save():
            dsc_s[...] = dsn[NC - 1]

        return dict(D=d_job, Q=q_job, V=v_job, K=k_job, save=save)

    SYNC = 8
    SK0 = 4
    SK1 = 4
    G = NQ * NC

    def att_emit(i, fwd, bwd):
        pend = []
        extra = []
        if fwd:
            F = [fwd_ctx(i, k) for k in range(NQ)]
        if bwd:
            Bk = [bwd_ctx(i - 1, k) for k in range(NQ)]
            Fc = fwd_ctx(i - 1, NQ - 1)
            pend += fwd_ctx(i - 1, NQ - 2)['fin']
            if isinstance(i, int):
                Bc = bwd_ctx(i - 2, NQ - 1)
            else:
                Bc = bwd_ctx(jnp.maximum(i - 2, 0), NQ - 1, valid=i >= 2)
        if fwd and bwd:
            k0 = jnp.minimum(2 * i - 2, NU // 2 - 2)
            extra = conv_ops(k0, 0) + conv_ops(k0, 1) + conv_ops(k0 + 1, 0) + conv_ops(k0 + 1, 1)
        tick = make_pacer(extra, (2 * G - SK0 - SK1) * SYNC)
        fgap = 4 if (fwd and bwd) else 2
        njob = [0]

        def hook(val):
            njob[0] += 1
            for k in range(SYNC):
                r = k * (CK // SYNC)
                if pend and k % fgap == fgap - 1:
                    make_pacer([(1, pend.pop(0))], 1)(val, r)
                if njob[0] > SK0:
                    tick(val, r)

        lag = 1 if bwd else 2
        for g in range(G):
            s, c = g % NQ, g // NQ
            sp, cp_ = (g - 1) % NQ, (g - 1) // NQ
            if bwd:
                Bk[s]['D'](c, hook)
                Bk[s]['V'](c)
                (Bc if g == 0 else Bk[sp])['K'](NC - 1 if g == 0 else cp_)
            if fwd:
                F[s]['S'](c, hook)
            if bwd and g == 0:
                Fc['O'](NC - 1)
                pend += Fc['fin']
            if fwd and g >= lag:
                so, co = (g - lag) % NQ, (g - lag) // NQ
                F[so]['O'](co)
                if co == NC - 1 and so < NQ - 2:
                    pend += F[so]['fin']
            if bwd:
                (Bc if g == 0 else Bk[sp])['Q'](NC - 1 if g == 0 else cp_)
        if not bwd:
            F[NQ - 2]['O'](NC - 1)
        for op in pend:
            op()
        if bwd and fwd:
            Bk[NQ - 1]['save']()
        if not fwd:
            Bk[NQ - 1]['K'](NC - 1)
            Bk[NQ - 1]['Q'](NC - 1)

    att_emit(0, True, False)

    def att_body(i, carry):
        att_emit(i, True, True)
        return carry

    lax.fori_loop(1, H, att_body, 0)
    att_emit(H, False, True)

    gx_v = x_v

    RS = 16
    PK0 = 24
    PK1 = 24

    def post_chunk(n, k, slot):
        f_even = finv_ref[0:C // 2, :]
        f_odd = finv_ref[C // 2:C, :]
        grp = pl.ds(pl.multiple_of(n * TN, TN), TN)
        sgrp = pl.ds(pl.multiple_of(n * 2 * TN, 2 * TN), 2 * TN)
        av, aq, ga, ak, ks = (r.at[grp, :] for r in (av_v, aq_v, ga_v, ak_v, ks_s))
        ops = []
        for dt in range(ND):
            ln = lanes(dt)
            sg = slot * ND + dt
            nx = ((slot + 3) % 4) * ND + dt
            for j, ref in enumerate((dxsp_s, ysp_s, dhsp_s)):
                rv = ref.at[sgrp, :]
                sp_s[sg, pl.ds(j * C, C // 2, stride=2), :] = _dot(f_even, rv[k * 2 * C:k * 2 * C + C, ln])
                sp_s[sg, pl.ds(j * C + 1, C // 2, stride=2), :] = _dot(f_odd, rv[k * 2 * C + C:(k + 1) * 2 * C, ln])
            acc = {}

            def mk(r0, dt=dt, ln=ln, sg=sg, nx=nx, acc=acc):
                def op():
                    rr = slice(k * C + r0, k * C + r0 + RS)
                    taps = shift_ref[:, ln].astype(f32)
                    nxt = sp_s[nx, 3 * C:3 * C + 8, :] if r0 == C - RS else acc['nxt']
                    dkv = sp_s[sg, r0:r0 + RS, :]
                    y = sp_s[sg, C + r0:C + r0 + RS, :]
                    dks = dkv * av[rr, ln].astype(f32)
                    av[rr, ln] = (dkv * ks[rr, ln].astype(f32)).astype(bf16)
                    aq[rr, ln] = (aq[rr, ln].astype(f32) * y).astype(bf16)
                    ga[rr, ln] = (ga[rr, ln].astype(f32) * y).astype(bf16)
                    acc['nxt'] = dks[0:8]
                    if r0 == 0:
                        sp_s[sg, 3 * C:3 * C + 8, :] = dks[0:8]
                    ext = jnp.concatenate([dks, nxt], axis=0)
                    kk = ak[rr, ln].astype(f32)
                    gk = None
                    for j in range(KS):
                        sh = dks if j == 0 else pltpu.roll(ext, RS + 8 - j, 0)[0:RS]
                        t = sh * taps[j:j + 1]
                        gk = t if gk is None else gk + t
                        pr = jnp.sum((sh * kk).reshape(RS // 8, 8, 128), axis=0)
                        acc[j] = pr if j not in acc else acc[j] + pr
                    ak[rr, ln] = gk.astype(bf16)
                    if r0 == 0:
                        for j in range(KS):
                            sacc_s[j, :, ln] += acc[j]
                return op

            def mkh(ln=ln, sg=sg):
                def op():
                    dh = sp_s[sg, 2 * C:3 * C, :]
                    sacc_s[KS, :, ln] = dh[0:8]
                    ssmk_v.at[:, grp][ln, k * C:(k + 1) * C] = dh.astype(bf16).T
                return op

            ops.append((16, mkh()))
            for r0 in range(C - RS, -1, -RS):
                ops.append((RS, mk(r0)))
        return ops

    for dt in range(ND):
        sp_s[3 * ND + dt, 3 * C:3 * C + 8, :] = jnp.zeros((8, 128), f32)

    def gx_body(i, carry):
        n = S // TN - 1 - i
        grp = pl.ds(pl.multiple_of(n * TN, TN), TN)
        for slot in range(TN // C):
            k = TN // C - 1 - slot
            tick = make_pacer(post_chunk(n, k, slot), 4 * (D // 8) - PK0 - PK1)
            cs = slice(k * C, (k + 1) * C)
            w = jnp.concatenate([(dq_s.at[:, grp][:, cs] * SCALE).astype(bf16),
                                 (dk_s.at[:, grp][:, cs] * LN2).astype(bf16),
                                 dv_s.at[:, grp][:, cs].astype(bf16)], axis=0)
            res = None
            for kg in range(4):
                ksl = slice(kg * 512, min((kg + 1) * 512, 3 * D))
                part = _dot(wqkv_v[:, ksl], w[ksl, :])
                for r8 in range(D // 8):
                    if kg * (D // 8) + r8 >= PK0:
                        tick(part, r8 * 8)
                res = part if res is None else res + part
            gx_v.at[grp, :][cs, :] = res.astype(bf16).T
        r = pl.ds(pl.multiple_of(n * TN, TN), TN)
        ro = pl.ds(pl.multiple_of(n * 2 * TN, TN), TN)
        ysp_s[ro, :] = _dot(ot_s[:, r].astype(bf16).T, wo_v[...]).astype(bf16)
        cp(aq_v.at[r, :], out_hbm.at[0, r, 0:D], sem_out.at[0]).start()
        cp(ga_v.at[r, :], gq_hbm.at[0, r, :], sem_out.at[1]).start()
        cp(ak_v.at[r, :], gk_hbm.at[0, r, :], sem_out.at[2]).start()
        cp(av_v.at[r, :], gv_hbm.at[0, r, :], sem_out.at[3]).start()
        cp(ssmk_v.at[:, r], gssmk_hbm.at[:, r], sem_out.at[4]).start()
        cp(gx_v.at[r, :], gx_hbm.at[0, r, :], sem_out.at[5]).start()
        cp(ysp_s.at[ro, :], out_hbm.at[0, r, D:2 * D], sem_out.at[6]).start()
        return carry

    lax.fori_loop(0, S // TN, gx_body, 0)
    o_oa = cp(aq_v, out_hbm.at[0, :, 0:D], sem_out.at[0])
    o_gq = cp(ga_v, gq_hbm.at[0], sem_out.at[1])
    o_gk = cp(ak_v, gk_hbm.at[0], sem_out.at[2])
    o_gv = cp(av_v, gv_hbm.at[0], sem_out.at[3])
    o_gs = cp(ssmk_v, gssmk_hbm, sem_out.at[4])
    o_gx = cp(gx_v, gx_hbm.at[0], sem_out.at[5])
    o_ob = cp(ysp_s.at[0:S, :], out_hbm.at[0, :, D:2 * D], sem_out.at[6])
    shift_ref[...] = jnp.sum(sacc_s[0:KS], axis=1).astype(bf16)
    ssmd_ref[...] = sacc_s[KS, 0, :].astype(bf16)
    o_sh = cp(shift_ref, gshift_hbm, sem_out.at[9])
    o_sd = cp(ssmd_ref, gssmd_hbm, sem_out.at[10])
    o_sh.start()
    o_sd.start()

    def gw_body(n, c):
        r = pl.ds(pl.multiple_of(n * 128, 128), 128)
        w = jnp.concatenate([(dq_s[r, :] * SCALE).astype(bf16),
                             (dk_s[r, :] * LN2).astype(bf16),
                             dv_s[r, :].astype(bf16)], axis=0)
        res = _dot(xt_s[...], w, NT).astype(bf16)
        for j in range(3):
            wqkv_v[:, pl.ds(pl.multiple_of(j * D + n * 128, 128), 128)] = res[:, lanes(j)]
        wo_v[:, r] = _dot(ot_s[...].astype(bf16), gb_v[:, r]).astype(bf16)
        for j in range(3):
            cj = pl.ds(pl.multiple_of(j * D + n * 128, 128), 128)
            cp(wqkv_v.at[:, cj], gwqkv_hbm.at[:, cj], sem_out.at[7]).start()
        cp(wo_v.at[:, r], gwo_hbm.at[:, r], sem_out.at[8]).start()
        return c

    lax.fori_loop(0, ND, gw_body, 0)
    o_gw = cp(wqkv_v, gwqkv_hbm, sem_out.at[7])
    o_gwo = cp(wo_v, gwo_hbm, sem_out.at[8])
    for o in (o_oa, o_gq, o_gk, o_gv, o_gs, o_sh, o_sd, o_gx, o_ob, o_gw, o_gwo):
        o.wait()


@jax.jit
def pallas_concat_heads__ssm_conv_h3__softmax_full_mha__prompt_kernel(
    A_q: jax.Array,
    A_k: jax.Array,
    A_v: jax.Array,
    A_shift_k: jax.Array,
    A_ssm_k: jax.Array,
    A_ssm_D: jax.Array,
    B_x: jax.Array,
    B_wqkv: jax.Array,
    B_wo: jax.Array,
    grad_out: jax.Array,
):
    fwd_np, inv_np = _dft_mats()
    fmat = jnp.asarray(fwd_np, dtype=bf16)
    finv = jnp.asarray(inv_np, dtype=bf16)

    hbm = pl.BlockSpec(memory_space=pl.ANY)
    sds = jax.ShapeDtypeStruct
    out_shape = (
        sds((1, S, 2 * D), bf16),
        sds((1, S, D), bf16),
        sds((1, S, D), bf16),
        sds((1, S, D), bf16),
        sds((KS, D), bf16),
        sds((D, S), bf16),
        sds((D,), bf16),
        sds((1, S, D), bf16),
        sds((D, 3 * D), bf16),
        sds((D, D), bf16),
    )
    scratch = [
        pltpu.VMEM((S, D), bf16),
        pltpu.VMEM((D, 3 * D), bf16),
        pltpu.VMEM((D, D), bf16),
        pltpu.VMEM((S, D), bf16),
        pltpu.VMEM((S, D), bf16),
        pltpu.VMEM((S, D), bf16),
        pltpu.VMEM((S, D), bf16),
        pltpu.VMEM((S, D), bf16),
        pltpu.VMEM((D, S), bf16),
        pltpu.VMEM((D, S), bf16),
        pltpu.VMEM((D, S), f32),
        pltpu.VMEM((D, S), f32),
        pltpu.VMEM((D, S), f32),
        pltpu.VMEM((D, S), f32),
        pltpu.VMEM((D, S), f32),
        pltpu.VMEM((D, S), f32),
        pltpu.VMEM((NP, S, 128), bf16),
        pltpu.VMEM((S, TQ), bf16),
        pltpu.VMEM((S, TQ), bf16),
        pltpu.VMEM((S, TQ), bf16),
        pltpu.VMEM((S, TQ), bf16),
        pltpu.VMEM((NB * 2 * C, D), bf16),
        pltpu.VMEM((NB * 2 * C, D), bf16),
        pltpu.VMEM((NB * 2 * C, D), bf16),
        pltpu.VMEM((NU + 3, SPK * NB * 8, 128), f32),
        pltpu.VMEM((H * 8, S), f32),
        pltpu.VMEM((NQ, 64, TQ), bf16),
        pltpu.VMEM((NQ, WIN, TQ), f32),
        pltpu.VMEM((2 * NQ, WIN, TQ), f32),
        pltpu.VMEM((CK, TQ), bf16),
        pltpu.VMEM((2 * C, C), bf16),
        pltpu.VMEM((C, C), bf16),
        pltpu.VMEM((KS + 1, 8, D), f32),
        pltpu.VMEM((KS, D), bf16),
        pltpu.VMEM((D,), bf16),
        pltpu.SMEM((1,), jnp.int32),
        pltpu.SemaphoreType.DMA((23,)),
        pltpu.SemaphoreType.DMA((11,)),
    ]
    outs = pl.pallas_call(
        _kernel,
        out_shape=out_shape,
        in_specs=[hbm] * 12,
        out_specs=(hbm,) * 10,
        scratch_shapes=scratch,
        compiler_params=pltpu.CompilerParams(vmem_limit_bytes=127 * 1024 * 1024),
    )(A_q, A_k, A_v, A_shift_k.T, A_ssm_k, A_ssm_D, B_x, B_wqkv, B_wo, grad_out, fmat, finv)
    outs = list(outs)
    outs[4] = outs[4].T
    return tuple(outs)
```

```python
import functools
import math

import numpy as np
import jax
import jax.numpy as jnp
from jax import lax
import jax.experimental.pallas as pl
import jax.experimental.pallas.tpu as pltpu

f32 = jnp.float32
bf16 = jnp.bfloat16

S = 2048
D = 640
H = 32
DH = 20
KS = 4
C = 128
NB = S // C
ND = D // 128
TQ = 512
NQ = S // TQ
NT_ALL = H * NQ
CK = 128
NC = S // CK
WIN = 24
NP = H // 2
NU = (C // 8) * ND
SPK = 6
TN = 512
SCALE = DH ** -0.5
LOG2E = math.log2(math.e)
LN2 = math.log(2.0)
SAFE_BOUND = 16.0

mul, add, sub = lax.mul, lax.add, lax.sub

NN = (((1,), (0,)), ((), ()))
NT = (((1,), (1,)), ((), ()))


def _dot(a, b, dims=NN):
    return lax.dot_general(a, b, dims, preferred_element_type=f32)


def _dft_mats():
    hf = C // 2
    f = np.concatenate([np.arange(hf), C - 1 - np.arange(hf)]).astype(np.float64)[:, None]
    u = np.arange(C, dtype=np.float64)[None, :]
    ang = np.pi * (2.0 * f + 1.0) * u / (2.0 * C)
    fwd = np.concatenate([np.cos(ang), -np.sin(ang)], axis=0)
    half = np.concatenate([np.cos(ang[:hf]), -np.sin(ang[:hf])], axis=0).T / C
    inv = np.concatenate([half[0::2], half[1::2]], axis=0)
    return fwd.astype(np.float32), inv.astype(np.float32)


def _v8(i):
    return slice(8 * i, 8 * i + 8)


def _kernel(aq_hbm, ak_hbm, av_hbm, shift_hbm, ssmk_hbm, ssmd_hbm, x_hbm, wqkv_hbm, wo_hbm, g_hbm,
            f_hbm, finv_hbm,
            out_hbm, gq_hbm, gk_hbm, gv_hbm, gshift_hbm, gssmk_hbm, gssmd_hbm, gx_hbm, gwqkv_hbm, gwo_hbm,
            x_v, wqkv_v, wo_v, gb_v, ga_v, aq_v, ak_v, av_v, ssmk_v, xt_s,
            qt_s, kt_s, vt_s, dot_s, dk_s, dv_s, kvg_s, pa_s, pb_s, pc_s, pd_s,
            ysp_s, dxsp_s, dhsp_s, sp_s, fb_s, m_s,
            wdo_s, dos_s, acc_s, dsc_s, f_ref, finv_ref, sacc_s, shift_ref, ssmd_ref,
            zero_s, sem):

    def cp(src, dst, sem):
        return pltpu.make_async_copy(src, dst, sem)

    def c_x(n):
        r = pl.ds(pl.multiple_of(n * TN, TN), TN)
        return cp(x_hbm.at[0, r, :], x_v.at[r, :], sem.at[n])

    def c_gb(n):
        r = pl.ds(pl.multiple_of(n * TN, TN), TN)
        return cp(g_hbm.at[0, r, D:2 * D], gb_v.at[r, :], sem.at[4 + n])

    WH = 1024
    c_wa = cp(wqkv_hbm.at[:, 0:WH], wqkv_v.at[:, 0:WH], sem.at[8])
    c_wb = cp(wqkv_hbm.at[:, WH:3 * D], wqkv_v.at[:, WH:3 * D], sem.at[9])
    c_wo = cp(wo_hbm, wo_v, sem.at[10])
    c_a = [cp(src, dst, sem.at[11]) for src, dst in (
        (shift_hbm, shift_ref), (ssmd_hbm, ssmd_ref), (f_hbm, f_ref), (finv_hbm, finv_ref),
        (ssmk_hbm, ssmk_v), (g_hbm.at[0, :, 0:D], ga_v), (aq_hbm.at[0], aq_v),
        (ak_hbm.at[0], ak_v), (av_hbm.at[0], av_v))]
    sem_out = sem.at[12]

    c_gb(0).start()
    c_wo.start()
    for cc in (c_gb(1), c_gb(2), c_wa, c_gb(3), c_wb):
        cc.start()
    for n in range(S // TN):
        c_x(n).start()
    for cc in c_a:
        cc.start()

    wt_s = dxsp_s
    ks_s = x_v
    dq_s = qt_s
    ot_s = dot_s

    def zero_body(n, c):
        cols = pl.ds(pl.multiple_of(n * 128, 128), 128)
        dk_s[:, cols] = jnp.zeros((D, 128), f32)
        dv_s[:, cols] = jnp.zeros((D, 128), f32)
        m_s[:, cols] = jnp.zeros((H * 8, 128), f32)
        return c

    lax.fori_loop(0, S // 128, zero_body, 0)
    dsc_s[...] = jnp.zeros((CK, TQ), bf16)
    acc_s[...] = jnp.zeros((2 * NQ, WIN, TQ), f32)
    sacc_s[...] = jnp.zeros((KS + 1, 8, D), f32)
    zero_s[0] = 0

    def do_chunk(n):
        cols = pl.ds(pl.multiple_of(n * TN, TN), TN)
        dot_s[:, cols] = _dot(wo_v[...], gb_v[cols, :], NT)

    def do0_body(n, c):
        c_gb(n).wait()
        do_chunk(n)
        return c

    def do1_body(n, c):
        c_gb(n).wait()

        @pl.when(n == 2)
        def _():
            c_wa.wait()

        @pl.when(n == 3)
        def _():
            c_wb.wait()

        do_chunk(n)
        w0 = pl.multiple_of((n - 2) * (3 * D - WH), 128)
        wt_s[pl.ds(w0, WH), :] = wqkv_v[:, pl.ds(w0, WH)].T
        return c

    c_wo.wait()
    lax.fori_loop(0, 2, do0_body, 0)
    lax.fori_loop(2, 4, do1_body, 0)

    def proj_body(n, carry):
        qmax, kmax = carry
        c_x(n).wait()

        c0 = pl.multiple_of(n * TN, TN)
        xc = x_v[pl.ds(c0, TN), :]
        kt = _dot(wt_s[D:2 * D, :], xc, NT).astype(bf16).astype(f32)
        kt_s[:, pl.ds(c0, TN)] = kt
        vt = _dot(wt_s[2 * D:3 * D, :], xc, NT).astype(bf16).astype(f32)
        vt_s[:, pl.ds(c0, TN)] = vt
        ones = jnp.ones((8, TN), f32)
        zeros = jnp.zeros((40, TN), f32)
        for p in range(NP):
            blk = jnp.concatenate(
                [kt[40 * p:40 * p + 40], ones, vt[40 * p:40 * p + 40], zeros], axis=0).astype(bf16)
            kvg_s[p, pl.ds(c0, TN), :] = blk.T
        qt = (_dot(wt_s[0:D, :], xc, NT) * (SCALE * LOG2E)).astype(bf16).astype(f32)
        qt_s[:, pl.ds(c0, TN)] = qt
        xt_s[:, pl.ds(c0, TN)] = xc.T
        qa = jnp.max(jnp.abs(qt).reshape(D // 8, 8, TN), axis=0)
        ka = jnp.max(jnp.abs(kt).reshape(D // 8, 8, TN), axis=0)
        return jnp.maximum(qmax, qa), jnp.maximum(kmax, ka)

    qmax, kmax = lax.fori_loop(0, S // TN, proj_body,
                               (jnp.zeros((8, TN), f32), jnp.zeros((8, TN), f32)))

    for cc in c_a:
        cc.wait()

    def lanes(dt):
        return slice(dt * 128, (dt + 1) * 128)

    PRU = 8

    def pre_chunk(i, k):
        fmat = f_ref[...]
        taps = shift_ref[...].astype(f32)
        grp = pl.ds(pl.multiple_of(i * PRU * C, PRU * C), PRU * C)
        rows = slice(k * C, (k + 1) * C)
        av, aq, ga, ak, ks = (r.at[grp, :] for r in (av_v, aq_v, ga_v, ak_v, ks_s))
        spv = sp_s.at[:, pl.ds(pl.multiple_of(i * PRU * SPK * 8, PRU * SPK * 8), PRU * SPK * 8), :]

        def put(kk, dt, val):
            for part in range(2):
                spv[dt * 16:(dt + 1) * 16, _v8(SPK * k + 2 * kk + part), :] = (
                    val[part * C:(part + 1) * C, :].reshape(C // 8, 8, 128))

        hs = _dot(fmat, ssmk_v.at[:, grp][:, rows], NT)
        if k == 0:
            ssm_d = jnp.where(i == 0, ssmd_ref[...].astype(f32).reshape(1, D), 0.0)
            hs = jnp.concatenate([hs[0:C] + ssm_d, hs[C:2 * C]], axis=0)
        for dt in range(ND):
            put(1, dt, hs[:, lanes(dt)])
        for dt in range(ND):
            ln = lanes(dt)
            dy = (ga[rows, ln].astype(f32) * aq[rows, ln].astype(f32)).astype(bf16)
            put(2, dt, _dot(fmat, dy))
            kf = ak[rows, ln].astype(f32)
            if k == 0:
                h0 = pl.multiple_of(jnp.maximum(i * PRU * C - 16, 0), 16)
                halo = jnp.where(i > 0, ak_v[pl.ds(h0, 16), ln].astype(f32)[8:16], 0.0)
            else:
                halo = ak[k * C - 16:k * C, ln].astype(f32)[8:16]
            ext = jnp.concatenate([halo, kf], axis=0)
            ksh = kf * taps[0:1, ln]
            for j in range(1, KS):
                ksh = ksh + pltpu.roll(ext, j, 0)[8:8 + C] * taps[j:j + 1, ln]
            ks[rows, ln] = ksh.astype(bf16)
            put(0, dt, _dot(fmat, (ksh * av[rows, ln].astype(f32)).astype(bf16)))

    def pre_body(i, c):
        for k in range(PRU):
            pre_chunk(i, k)
        return jnp.max(qmax) * jnp.max(kmax) * float(DH)

    bound = lax.fori_loop(0, NB // PRU, pre_body, jnp.float32(0.0))

    def conv_ops(k, mirror):
        sgn = jnp.where(lax.broadcasted_iota(jnp.int32, (8, 128), 0) % 2 == mirror, 1.0, -1.0).astype(f32)
        dt = lax.shift_right_logical(k, 3)
        u = dt * 16 + (k & 7) + 8 * mirror
        r0 = pl.multiple_of((k & 7) * 8, 8)
        ll = pl.ds(pl.multiple_of(dt * 128, 128), 128)
        ops = []

        def ld(kb):
            k, b = kb
            return sp_s[u, _v8(SPK * b + 2 * k), :], sp_s[u, _v8(SPK * b + 2 * k + 1), :]

        def cm(a, b, conj):
            if conj:
                return add(mul(a[0], b[0]), mul(a[1], b[1])), sub(mul(a[0], b[1]), mul(a[1], b[0]))
            return sub(mul(a[0], b[0]), mul(a[1], b[1])), add(mul(a[0], b[1]), mul(a[1], b[0]))

        def st(ref, b, vr, vi):
            j = 2 * (ref[1] * NB + b)
            if not mirror:
                sp_s[NU + 1, _v8(j), :] = vr
                sp_s[NU + 1, _v8(j + 1), :] = vi
            else:
                zr, zi = sp_s[NU + 1, _v8(j), :], sp_s[NU + 1, _v8(j + 1), :]
                sp_s[NU + 1, _v8(j), :] = vr
                for q, v in enumerate((add(zr, vr), sub(zi, vi), sub(zr, vr), add(zi, vi))):
                    ro = b * 2 * C + q * (C // 2)
                    ref[0][ro:ro + 8, :] = v.astype(bf16)

        def add_group(outs, conj):
            accs = [None] * len(outs)
            cache = {}
            nt = max(len(t) for t, _ in outs)

            def mk(i):
                def op():
                    a = None
                    newc = {}
                    for oi, (terms, _) in enumerate(outs):
                        if i >= len(terms):
                            continue
                        ka, kb = terms[i]
                        if a is None:
                            a = ld(ka)
                        b = cache[kb] if kb in cache else ld(kb)
                        newc[kb] = b
                        t = cm(a, b, conj)
                        accs[oi] = t if accs[oi] is None else (add(accs[oi][0], t[0]), add(accs[oi][1], t[1]))
                    cache.clear()
                    cache.update(newc)
                    if i == nt - 1:
                        for oi, (_, fin) in enumerate(outs):
                            fin(*accs[oi])
                return op

            for i in range(nt):
                ops.append((sum(1 for t, _ in outs if i < len(t)), mk(i)))

        def fin_next(ref):
            prev = {}

            def mkfin(d):
                def fin(ar, ai):
                    if d > 0:
                        st(ref, d - 1, add(prev['r'], mul(sgn, ai)), sub(prev['i'], mul(sgn, ar)))
                    if d == NB - 1:
                        st(ref, d, ar, ai)
                    prev['r'], prev['i'] = ar, ai
                return fin
            return mkfin

        def fin_prev(ref):
            prev = {}

            def mkfin(b):
                def fin(ar, ai):
                    if b > 0:
                        st(ref, b, sub(ar, mul(sgn, prev['i'])), add(ai, mul(sgn, prev['r'])))
                    else:
                        st(ref, b, ar, ai)
                    prev['r'], prev['i'] = ar, ai
                return fin
            return mkfin

        X, G, Y = 0, 1, 2
        BLK = 2
        vh, vy, vx = (r.at[pl.ds(r0, NB * 2 * C - 56), ll] for r in (dhsp_s, ysp_s, dxsp_s))
        fh, fy, fx = fin_next((vh, 0)), fin_prev((vy, 1)), fin_next((vx, 2))
        kinds = [(lambda d: [((X, j), (Y, j + d)) for j in range(NB - d)], fh, True),
                 (lambda b: [((G, d), (X, b - d)) for d in range(b + 1)], fy, False),
                 (lambda b: [((G, d), (Y, b + d)) for d in range(NB - b)], fx, True)]
        for terms_of, fin, conj in kinds:
            for o0 in range(0, NB, BLK):
                add_group([(terms_of(o), fin(o)) for o in range(o0, o0 + BLK)], conj)
        return ops

    def make_pacer(extra, npts, ref=None, unit=NU):
        ref = sp_s if ref is None else ref
        tot = sum(w for w, _ in extra)
        zero = zero_s[0]
        sink_u = zero + unit
        sink_r = pl.ds(pl.multiple_of(zero, 8), 8)
        pos = dict(i=0, w=0, pt=0)

        def tick(val, r):
            pos['pt'] += 1
            lim = pos['pt'] * tot / npts
            if pos['i'] < len(extra) and pos['w'] < lim:
                ref[sink_u, sink_r, :] = val[r:r + 8, 0:128]
            while pos['i'] < len(extra) and pos['w'] < lim:
                w, op = extra[pos['i']]
                op()
                pos['i'] += 1
                pos['w'] += w

        tick.done = lambda: pos['i'] == len(extra)
        return tick

    def iota(n, m):
        return lax.broadcasted_iota(jnp.int32, (n, m), 0)

    def head_idx(h):
        if isinstance(h, int):
            par, pair = h % 2, h // 2
            return par, pair, pair * 40 + par * 16, pair * 40, h * 8
        par = h & 1
        pair = lax.shift_right_logical(h, 1)
        return (par, pair, pl.multiple_of(pair * 40 + par * 16, 8), pl.multiple_of(pair * 40, 8),
                pl.multiple_of(h * 8, 8))

    def make_wq(h, qcols):
        par, pair, w0, p0, m0 = head_idx(h)
        row40 = iota(40, TQ)
        qp = qt_s[pl.ds(p0, 40), qcols]
        qp = jnp.where((row40 >= par * DH) & (row40 < par * DH + DH), qp, 0.0)
        top = jnp.concatenate([qp, m_s[pl.ds(m0, 8), qcols]], axis=0).astype(bf16)
        return jnp.concatenate([top, jnp.zeros((80, TQ), bf16)], axis=0)

    @pl.when(jnp.logical_not(bound <= SAFE_BOUND))
    def _():
        def max_body(t, c):
            h = lax.shift_right_logical(t, 2)
            par, pair, w0, p0, m0 = head_idx(h)
            qcols = pl.ds(pl.multiple_of((t & 3) * TQ, TQ), TQ)
            wq = make_wq(h, qcols)

            def inner(ci, m):
                k0 = pl.multiple_of(ci * 256, 256)
                s = _dot(kvg_s[pair, pl.ds(k0, 256), :], wq)
                return jnp.maximum(m, jnp.max(s.reshape(32, 8, TQ), axis=0))

            m = lax.fori_loop(0, S // 256, inner, jnp.full((8, TQ), -jnp.inf, f32))
            nm = -jnp.max(m, axis=0, keepdims=True)
            hi = nm.astype(bf16).astype(f32)
            mid = (nm - hi).astype(bf16).astype(f32)
            lo = nm - hi - mid
            row8 = iota(8, TQ)
            m_s[pl.ds(m0, 8), qcols] = jnp.where(
                row8 == 0, hi, jnp.where(row8 == 1, mid, jnp.where(row8 == 2, lo, 0.0)))
            return c

        lax.fori_loop(0, NT_ALL, max_body, 0)

    def rows_of(c):
        return slice(c * CK, (c + 1) * CK)

    P_S = (pa_s, pb_s, pc_s, pd_s)

    def fwd_ctx(h, sid, c0=0):
        par, pair, w0, p0, m0 = head_idx(h)
        p_s = P_S[sid]
        acc_ref = acc_s.at[sid]
        lz = {}
        onek = iota(WIN, CK) == (1 - par) * DH
        ones_k = jnp.ones((WIN, CK), f32)
        pn = {}

        def s_job(c, hook):
            if 'wq' not in lz:
                lz['wq'] = make_wq(h, slice(sid * TQ, (sid + 1) * TQ))
            s = _dot(kvg_s[pair, rows_of(c), :], lz['wq'])
            hook(s)
            p = lax.exp2(s).astype(bf16)
            p_s[rows_of(c), :] = p
            pn[c] = p

        def o_job(c):
            vw = lax.select(onek, ones_k, vt_s[pl.ds(w0, WIN), rows_of(c)])
            r = _dot(vw, pn[c] if c in pn else p_s[rows_of(c), :])
            if c == c0:
                acc_ref[...] = r
            elif c < NC - 1:
                acc_ref[...] = add(acc_ref[...], r)
            else:
                oacc = acc_ref[...] + r
                for qt in range(TQ // 128):
                    o0 = (sid * 4 + qt) * WIN
                    sp_s[NU + 2, o0:o0 + WIN, :] = oacc[:, lanes(qt)]

        rl0 = 16 * WIN + sid * 64

        def oacc_ld(q0, n):
            return jnp.concatenate([sp_s[NU + 2, (sid * 4 + qt) * WIN:(sid * 4 + qt + 1) * WIN, :]
                                    for qt in range(q0, q0 + n)], axis=1)

        def row_ld(r0, q0, n):
            return jnp.concatenate([sp_s[NU + 2, r0 + qt * 8:r0 + qt * 8 + 8, :]
                                    for qt in range(q0, q0 + n)], axis=1)

        def fin_a():
            oacc = oacc_ld(0, 4)
            rl = 1.0 / jnp.where(par == 0, oacc[DH:DH + 1], oacc[0:1])
            for qt in range(4):
                sp_s[NU + 2, rl0 + qt * 8:rl0 + qt * 8 + 8, :] = jnp.broadcast_to(rl[:, lanes(qt)], (8, 128))

        def fin_b(q0):
            def op():
                row24 = iota(WIN, 256)
                rl = jnp.concatenate([row_ld(rl0, q0, 2)] * 3, axis=0)
                ws = slice(q0 * 128, q0 * 128 + 256)
                cs = slice(sid * TQ + q0 * 128, sid * TQ + q0 * 128 + 256)
                msk = (row24 >= par * 4) & (row24 < par * 4 + DH)
                o = oacc_ld(q0, 2) * rl
                dow = dot_s[pl.ds(w0, WIN), cs]
                dosn = jnp.where(msk, dow * rl, 0.0).astype(bf16).astype(f32)
                pr = dosn * o
                pr = pr[0:8] + pr[8:16] + pr[16:24]
                for j in range(2):
                    r0 = rl0 + 32 + (q0 + j) * 8
                    sp_s[NU + 2, r0:r0 + 8, :] = pr[:, lanes(j)]
                z8 = jnp.zeros((8, 256), f32)
                z16 = jnp.zeros((16, 256), f32)
                dop = jnp.where(par == 0, jnp.concatenate([dosn, z16], axis=0),
                                jnp.concatenate([z16, dosn], axis=0))
                wdo_s[sid, 16:64, ws] = jnp.concatenate([dop, z8], axis=0).astype(bf16)
                dos_s[sid, :, ws] = dosn
                ot_s[pl.ds(w0, WIN), cs] = jnp.where(msk, o, dow)
            return op

        def fin_c():
            row16 = iota(16, TQ)
            nd = -jnp.sum(row_ld(rl0 + 32, 0, 4), axis=0, keepdims=True)
            hi = nd.astype(bf16).astype(f32)
            wdo_s[sid, 0:16, :] = jnp.where(row16 == 8, hi, jnp.where(row16 == 9, nd - hi, 0.0)).astype(bf16)

        def stage_q():
            qcols = slice(sid * TQ, (sid + 1) * TQ)
            qv = qt_s[pl.ds(w0, WIN), qcols]
            mr = m_s[pl.ds(m0, 8), qcols]
            ini = mr[0:1] + mr[1:2] + mr[2:3]
            for qt in range(4):
                base = (sid * 4 + qt) * 40
                fb_s[4, pl.ds(base + 4 - 4 * par, WIN), :] = qv[:, lanes(qt)]
                fb_s[4, base + 32:base + 40, :] = jnp.broadcast_to(ini[:, lanes(qt)], (8, 128))

        def vpu_ops():
            ops = []
            for kb in range(CK // 16):
                for q0 in (0, 2):
                    acc = {}

                    def mk(d, kb=kb, q0=q0, acc=acc):
                        def op():
                            r0 = (d % 6) * CK + kb * 16
                            kv = fb_s[d // 6, r0:r0 + 16, :]
                            for qt in (q0, q0 + 1):
                                base = (sid * 4 + qt) * 40
                                t = mul(kv, fb_s[4, base + 4 + d:base + 5 + d, :])
                                acc[qt] = add(t, fb_s[4, base + 32:base + 33, :] if d == 0 else acc[qt])
                            if d == DH - 1:
                                a = jnp.concatenate([acc[q0], acc[q0 + 1]], axis=1)
                                p_s[kb * 16:kb * 16 + 16, q0 * 128:q0 * 128 + 256] = lax.exp2(a).astype(bf16)
                        return op

                    ops += [(1, mk(d)) for d in range(DH)]
            return ops

        return dict(S=s_job, O=o_job, fin=[fin_a, fin_b(0), fin_b(2), fin_c], stage=stage_q, vpu=vpu_ops)

    def stage_k(h):
        par, pair, w0, p0, m0 = head_idx(h)
        fb_s[4, pl.ds(644 - 4 * par, WIN), :] = kt_s[pl.ds(w0, WIN), 0:CK]
        for d in range(DH):
            row = fb_s[4, 644 + d:645 + d, :]
            fb_s[d // 6, (d % 6) * CK:(d % 6 + 1) * CK, :] = jnp.broadcast_to(row, (128, CK)).T

    def bwd_ctx(h, sid, valid=None):
        par, pair, w0, p0, m0 = head_idx(h)
        p_s = P_S[sid]
        acc_ref = acc_s.at[NQ + sid]
        qcols = slice(sid * TQ, (sid + 1) * TQ)
        row24 = iota(WIN, TQ)
        msk = (row24 >= par * 4) & (row24 < par * 4 + DH)
        lz = {}
        dsn = {}

        def d_job(c, hook):
            if 'wdo' not in lz:
                z32 = jnp.zeros((32, TQ), bf16)
                lz['wdo'] = jnp.concatenate([z32, wdo_s[sid], z32], axis=0)
            dp = _dot(kvg_s[pair, rows_of(c), :], lz['wdo'])
            hook(dp)
            dsn[c] = mul(p_s[rows_of(c), :].astype(f32), dp).astype(bf16)

        def getds(c):
            return dsn[c] if c in dsn else dsc_s[...]

        def q_job(c):
            r = _dot(kt_s[pl.ds(w0, WIN), rows_of(c)], getds(c))
            if c == 0:
                acc_ref[...] = r
            elif c < NC - 1:
                acc_ref[...] = add(acc_ref[...], r)
            else:
                mk = msk if valid is None else (msk & valid)
                dq_s[pl.ds(w0, WIN), qcols] = jnp.where(mk, acc_ref[...] + r, dq_s[pl.ds(w0, WIN), qcols])

        def v_job(c):
            if 'dos' not in lz:
                lz['dos'] = dos_s[sid]
            dv_s[pl.ds(w0, WIN), rows_of(c)] = add(dv_s[pl.ds(w0, WIN), rows_of(c)],
                                                   _dot(lz['dos'], p_s[rows_of(c), :], NT))

        def k_job(c):
            if 'qw' not in lz:
                lz['qw'] = jnp.where(msk, qt_s[pl.ds(w0, WIN), qcols], 0.0)
            dk_s[pl.ds(w0, WIN), rows_of(c)] = add(dk_s[pl.ds(w0, WIN), rows_of(c)],
                                                   _dot(lz['qw'], getds(c), NT))

        def save():
            dsc_s[...] = dsn[NC - 1]

        return dict(D=d_job, Q=q_job, V=v_job, K=k_job, save=save)

    SYNC = 8
    G = NQ * NC
    NCV = 3
    HCV = H - (NU // 2 + NCV - 1) // NCV
    PG = 56
    PL = 3

    def att_emit(i, fwd, bwd, mode=None):
        pend = []
        off = mode == 'vpu'
        if fwd:
            F = [fwd_ctx(i, k, 1 if off else 0) for k in range(NQ)]
        if bwd:
            Bk = [bwd_ctx(i - 1, k) for k in range(NQ)]
            Fc = fwd_ctx(i - 1, NQ - 1)
            pend += fwd_ctx(i - 1, NQ - 2)['fin']
            if isinstance(i, int):
                Bc = bwd_ctx(i - 2, NQ - 1)
            else:
                Bc = bwd_ctx(jnp.maximum(i - 2, 0), NQ - 1, valid=i >= 2)
        sk0 = 5 if off else 4
        if mode == 'conv':
            k0 = jnp.minimum(NCV * (i - HCV), NU // 2 - NCV)
            extra = sum([conv_ops(k0 + j, 0) + conv_ops(k0 + j, 1) for j in range(NCV)], [])
            tick = make_pacer(extra, (2 * G - sk0 - 4) * SYNC)
        elif off:
            extra = sum([F[k]['vpu']() for k in range(NQ)], [])
            tick = make_pacer(extra, (2 * PG - NQ - sk0) * SYNC, fb_s, 5)
        else:
            tick = make_pacer([], 1)
        prep = off or not bwd
        pg = PG if bwd else 8
        njob = [0]
        pull = [False]

        def hook(val):
            njob[0] += 1
            fgap = 4 if (fwd and bwd and not (off and njob[0] <= 8)) else 2
            for k in range(SYNC):
                r = k * (CK // SYNC)
                if pend and k % fgap == fgap - 1:
                    make_pacer([(1, pend.pop(0))], 1)(val, r)
                if njob[0] > sk0:
                    tick(val, r)
            if pull[0]:
                pull[0] = False
                make_pacer([(1, lambda: None)], 1, fb_s, 5)(val, 0)

        lag = 1 if bwd else 2
        pl_ = PL if bwd else 3 * PL
        for g in range(G):
            s, c = g % NQ, g // NQ
            sp, cp_ = (g - 1) % NQ, (g - 1) // NQ
            if prep:
                if g == pg:
                    assert tick.done()
                    stage_k(i + 1)
                if g == pg + pl_:
                    pull[0] = True
                if pg + pl_ < g <= pg + pl_ + NQ:
                    fwd_ctx(i + 1, g - pg - pl_ - 1)['stage']()
                    pull[0] = True
            if bwd:
                assert g not in (NQ - 2, NQ - 1) or not pend
                Bk[s]['D'](c, hook)
                Bk[s]['V'](c)
                (Bc if g == 0 else Bk[sp])['K'](NC - 1 if g == 0 else cp_)
            if fwd and not (off and c == 0):
                F[s]['S'](c, hook)
            if off and c == NC - 2:
                F[s]['O'](0)
            if bwd and g == 0:
                Fc['O'](NC - 1)
                pend += Fc['fin']
            if fwd and g >= lag:
                so, co = (g - lag) % NQ, (g - lag) // NQ
                if not (off and co == 0):
                    F[so]['O'](co)
                if co == NC - 1 and so < NQ - 2:
                    pend += F[so]['fin']
            if bwd:
                (Bc if g == 0 else Bk[sp])['Q'](NC - 1 if g == 0 else cp_)
        if not bwd:
            F[NQ - 2]['O'](NC - 1)
        assert tick.done()
        for op in pend:
            op()
        if bwd and fwd:
            Bk[NQ - 1]['save']()
        if not fwd:
            Bk[NQ - 1]['K'](NC - 1)
            Bk[NQ - 1]['Q'](NC - 1)

    att_emit(0, True, False)

    def attv_body(i, carry):
        att_emit(i, True, True, 'vpu')
        return carry

    def attc_body(i, carry):
        att_emit(i, True, True, 'conv')
        return carry

    lax.fori_loop(1, HCV, attv_body, 0)
    lax.fori_loop(HCV, H, attc_body, 0)
    att_emit(H, False, True)

    gx_v = x_v

    RS = 32
    PK0 = 24
    PK1 = 24

    def post_chunk(n, k, slot):
        f_even = finv_ref[0:C // 2, :]
        f_odd = finv_ref[C // 2:C, :]
        grp = pl.ds(pl.multiple_of(n * TN, TN), TN)
        sgrp = pl.ds(pl.multiple_of(n * 2 * TN, 2 * TN), 2 * TN)
        av, aq, ga, ak, ks = (r.at[grp, :] for r in (av_v, aq_v, ga_v, ak_v, ks_s))
        ops = []
        for dt in range(ND):
            ln = lanes(dt)
            sg = slot * ND + dt
            nx = ((slot + 3) % 4) * ND + dt
            for j, ref in enumerate((dxsp_s, ysp_s, dhsp_s)):
                rv = ref.at[sgrp, :]
                sp_s[sg, pl.ds(j * C, C // 2, stride=2), :] = _dot(f_even, rv[k * 2 * C:k * 2 * C + C, ln])
                sp_s[sg, pl.ds(j * C + 1, C // 2, stride=2), :] = _dot(f_odd, rv[k * 2 * C + C:(k + 1) * 2 * C, ln])
            acc = {}

            def mk(r0, dt=dt, ln=ln, sg=sg, nx=nx, acc=acc):
                def op():
                    rr = slice(k * C + r0, k * C + r0 + RS)
                    taps = shift_ref[:, ln].astype(f32)
                    nxt = sp_s[nx, 3 * C:3 * C + 8, :] if r0 == C - RS else acc['nxt']
                    dkv = sp_s[sg, r0:r0 + RS, :]
                    y = sp_s[sg, C + r0:C + r0 + RS, :]
                    dks = mul(dkv, av[rr, ln].astype(f32))
                    av[rr, ln] = mul(dkv, ks[rr, ln].astype(f32)).astype(bf16)
                    aq[rr, ln] = mul(aq[rr, ln].astype(f32), y).astype(bf16)
                    ga[rr, ln] = mul(ga[rr, ln].astype(f32), y).astype(bf16)
                    acc['nxt'] = dks[0:8]
                    if r0 == 0:
                        sp_s[sg, 3 * C:3 * C + 8, :] = dks[0:8]
                    ext = jnp.concatenate([dks, nxt], axis=0)
                    kk = ak[rr, ln].astype(f32)
                    gk = None
                    for j in range(KS):
                        sh = dks if j == 0 else pltpu.roll(ext, RS + 8 - j, 0)[0:RS]
                        t = mul(sh, taps[j:j + 1])
                        gk = t if gk is None else add(gk, t)
                        pr = lax.reduce_sum(mul(sh, kk).reshape(RS // 8, 8, 128), (0,))
                        acc[j] = pr if j not in acc else add(acc[j], pr)
                    ak[rr, ln] = gk.astype(bf16)
                    if r0 == 0:
                        for j in range(KS):
                            sacc_s[j, :, ln] += acc[j]
                return op

            def mkh(ln=ln, sg=sg):
                def op():
                    dh = sp_s[sg, 2 * C:3 * C, :]
                    sacc_s[KS, :, ln] = dh[0:8]
                    ssmk_v.at[:, grp][ln, k * C:(k + 1) * C] = dh.astype(bf16).T
                return op

            ops.append((16, mkh()))
            for r0 in range(C - RS, -1, -RS):
                ops.append((RS, mk(r0)))
        return ops

    for dt in range(ND):
        sp_s[3 * ND + dt, 3 * C:3 * C + 8, :] = jnp.zeros((8, 128), f32)

    def gx_body(i, carry):
        n = S // TN - 1 - i
        grp = pl.ds(pl.multiple_of(n * TN, TN), TN)
        for slot in range(TN // C):
            k = TN // C - 1 - slot
            tick = make_pacer(post_chunk(n, k, slot), 4 * (D // 8) - PK0 - PK1)
            cs = slice(k * C, (k + 1) * C)
            w = jnp.concatenate([(dq_s.at[:, grp][:, cs] * SCALE).astype(bf16),
                                 (dk_s.at[:, grp][:, cs] * LN2).astype(bf16),
                                 dv_s.at[:, grp][:, cs].astype(bf16)], axis=0)
            res = None
            for kg in range(4):
                ksl = slice(kg * 512, min((kg + 1) * 512, 3 * D))
                part = _dot(wqkv_v[:, ksl], w[ksl, :])
                for r8 in range(D // 8):
                    if kg * (D // 8) + r8 >= PK0:
                        tick(part, r8 * 8)
                res = part if res is None else res + part
            assert tick.done()
            gx_v.at[grp, :][cs, :] = res.astype(bf16).T
        r = pl.ds(pl.multiple_of(n * TN, TN), TN)
        ro = pl.ds(pl.multiple_of(n * 2 * TN, TN), TN)
        ysp_s[ro, :] = _dot(ot_s[:, r].astype(bf16).T, wo_v[...]).astype(bf16)
        cp(aq_v.at[r, :], out_hbm.at[0, r, 0:D], sem_out).start()
        cp(ga_v.at[r, :], gq_hbm.at[0, r, :], sem_out).start()
        cp(ak_v.at[r, :], gk_hbm.at[0, r, :], sem_out).start()
        cp(av_v.at[r, :], gv_hbm.at[0, r, :], sem_out).start()
        cp(ssmk_v.at[:, r], gssmk_hbm.at[:, r], sem_out).start()
        cp(gx_v.at[r, :], gx_hbm.at[0, r, :], sem_out).start()
        cp(ysp_s.at[ro, :], out_hbm.at[0, r, D:2 * D], sem_out).start()
        return carry

    lax.fori_loop(0, S // TN, gx_body, 0)
    o_oa = cp(aq_v, out_hbm.at[0, :, 0:D], sem_out)
    o_gq = cp(ga_v, gq_hbm.at[0], sem_out)
    o_gk = cp(ak_v, gk_hbm.at[0], sem_out)
    o_gv = cp(av_v, gv_hbm.at[0], sem_out)
    o_gs = cp(ssmk_v, gssmk_hbm, sem_out)
    o_gx = cp(gx_v, gx_hbm.at[0], sem_out)
    o_ob = cp(ysp_s.at[0:S, :], out_hbm.at[0, :, D:2 * D], sem_out)
    shift_ref[...] = jnp.sum(sacc_s[0:KS], axis=1).astype(bf16)
    ssmd_ref[...] = sacc_s[KS, 0, :].astype(bf16)
    o_sh = cp(shift_ref, gshift_hbm, sem_out)
    o_sd = cp(ssmd_ref, gssmd_hbm, sem_out)
    o_sh.start()
    o_sd.start()

    def gw_body(n, c):
        r = pl.ds(pl.multiple_of(n * 128, 128), 128)
        w = jnp.concatenate([(dq_s[r, :] * SCALE).astype(bf16),
                             (dk_s[r, :] * LN2).astype(bf16),
                             dv_s[r, :].astype(bf16)], axis=0)
        res = _dot(xt_s[...], w, NT).astype(bf16)
        for j in range(3):
            wqkv_v[:, pl.ds(pl.multiple_of(j * D + n * 128, 128), 128)] = res[:, lanes(j)]
        wo_v[:, r] = _dot(ot_s[...].astype(bf16), gb_v[:, r]).astype(bf16)
        for j in range(3):
            cj = pl.ds(pl.multiple_of(j * D + n * 128, 128), 128)
            cp(wqkv_v.at[:, cj], gwqkv_hbm.at[:, cj], sem_out).start()
        cp(wo_v.at[:, r], gwo_hbm.at[:, r], sem_out).start()
        return c

    lax.fori_loop(0, ND, gw_body, 0)
    o_gw = cp(wqkv_v, gwqkv_hbm, sem_out)
    o_gwo = cp(wo_v, gwo_hbm, sem_out)
    for o in (o_oa, o_gq, o_gk, o_gv, o_gs, o_sh, o_sd, o_gx, o_ob, o_gw, o_gwo):
        o.wait()


@functools.partial(jax.jit, inline=True)
def pallas_concat_heads__ssm_conv_h3__softmax_full_mha__prompt_kernel(
    A_q: jax.Array,
    A_k: jax.Array,
    A_v: jax.Array,
    A_shift_k: jax.Array,
    A_ssm_k: jax.Array,
    A_ssm_D: jax.Array,
    B_x: jax.Array,
    B_wqkv: jax.Array,
    B_wo: jax.Array,
    grad_out: jax.Array,
):
    fwd_np, inv_np = _dft_mats()
    fmat = jnp.asarray(fwd_np, dtype=bf16)
    finv = jnp.asarray(inv_np, dtype=bf16)

    hbm = pl.BlockSpec(memory_space=pl.ANY)
    sds = jax.ShapeDtypeStruct
    out_shape = (
        sds((1, S, 2 * D), bf16),
        sds((1, S, D), bf16),
        sds((1, S, D), bf16),
        sds((1, S, D), bf16),
        sds((KS, D), bf16),
        sds((D, S), bf16),
        sds((D,), bf16),
        sds((1, S, D), bf16),
        sds((D, 3 * D), bf16),
        sds((D, D), bf16),
    )
    scratch = [
        pltpu.VMEM((S, D), bf16),
        pltpu.VMEM((D, 3 * D), bf16),
        pltpu.VMEM((D, D), bf16),
        pltpu.VMEM((S, D), bf16),
        pltpu.VMEM((S, D), bf16),
        pltpu.VMEM((S, D), bf16),
        pltpu.VMEM((S, D), bf16),
        pltpu.VMEM((S, D), bf16),
        pltpu.VMEM((D, S), bf16),
        pltpu.VMEM((D, S), bf16),
        pltpu.VMEM((D, S), f32),
        pltpu.VMEM((D, S), f32),
        pltpu.VMEM((D, S), f32),
        pltpu.VMEM((D, S), f32),
        pltpu.VMEM((D, S), f32),
        pltpu.VMEM((D, S), f32),
        pltpu.VMEM((NP, S, 128), bf16),
        pltpu.VMEM((S, TQ), bf16),
        pltpu.VMEM((S, TQ), bf16),
        pltpu.VMEM((S, TQ), bf16),
        pltpu.VMEM((S, TQ), bf16),
        pltpu.VMEM((NB * 2 * C, D), bf16),
        pltpu.VMEM((NB * 2 * C, D), bf16),
        pltpu.VMEM((NB * 2 * C, D), bf16),
        pltpu.VMEM((NU + 3, SPK * NB * 8, 128), f32),
        pltpu.VMEM((6, 768, 128), f32),
        pltpu.VMEM((H * 8, S), f32),
        pltpu.VMEM((NQ, 64, TQ), bf16),
        pltpu.VMEM((NQ, WIN, TQ), f32),
        pltpu.VMEM((2 * NQ, WIN, TQ), f32),
        pltpu.VMEM((CK, TQ), bf16),
        pltpu.VMEM((2 * C, C), bf16),
        pltpu.VMEM((C, C), bf16),
        pltpu.VMEM((KS + 1, 8, D), f32),
        pltpu.VMEM((KS, D), bf16),
        pltpu.VMEM((D,), bf16),
        pltpu.SMEM((1,), jnp.int32),
        pltpu.SemaphoreType.DMA((13,)),
    ]
    outs = pl.pallas_call(
        _kernel,
        out_shape=out_shape,
        in_specs=[hbm] * 12,
        out_specs=(hbm,) * 10,
        scratch_shapes=scratch,
        compiler_params=pltpu.CompilerParams(vmem_limit_bytes=127 * 1024 * 1024),
    )(A_q, A_k, A_v, A_shift_k.T, A_ssm_k, A_ssm_D, B_x, B_wqkv, B_wo, grad_out, fmat, finv)
    outs = list(outs)
    outs[4] = outs[4].T
    return tuple(outs)
```
